```python
import os as _os
_os.environ.setdefault('JAX_PLATFORMS', 'cpu')
import jax
import jax.numpy as jnp

def _softmax(x, axis=-1):
    return jax.nn.softmax(x, axis=axis)

def _gelu(x):
    return jax.nn.gelu(x, approximate=True)

def _silu(x):
    return jax.nn.silu(x)

def _sigmoid(x):
    return jax.nn.sigmoid(x)

def _layernorm(x, axis=-1, eps=1e-05):
    m = jnp.mean(x, axis=axis, keepdims=True)
    v = jnp.var(x, axis=axis, keepdims=True)
    return (x - m) / jnp.sqrt(v + eps)

def _scatter_add(tgt, idx, src, axis=0):
    return tgt.at[idx].add(src)

def _segment_sum(src, seg, n):
    return jax.ops.segment_sum(src, seg, n)

class _Rng:

    def __init__(self, key):
        self._k = key

    def _next(self):
        self._k, sub = jax.random.split(self._k)
        return sub

    def normal(self, shape):
        return jax.random.normal(self._next(), shape, dtype=jnp.bfloat16)

    def randint(self, lo, hi, shape):
        return jax.random.randint(self._next(), shape, lo, hi, dtype=jnp.int32)

    def uniform(self, shape, lo=0.0, hi=1.0):
        return jax.random.uniform(self._next(), shape, jnp.bfloat16, lo, hi)

    def permutation(self, n):
        return jax.random.permutation(self._next(), n)
kernel_name = 'sequential_preLN__memory_aug_recurrent_mem_tr__mixer_token_mlp__prompt'

def setup_inputs():
    _rng = _Rng(jax.random.key(int.from_bytes(__import__("os").urandom(4), "little")))
    _w = lambda a: (lambda t: t.astype(jnp.bfloat16) if jnp.issubdtype(t.dtype, jnp.floating) else t)(jnp.asarray(a))

    def _A_setup():
        B, S, Dm = (1, 2048, 448)
        H, Dh = (16, 256)
        M, seg = (8, 32)
        seg = min(seg, S)
        S = S // seg * seg
        return {'x': _w((lambda *s: _rng.normal(s) * 0.05)(B, S, Dm)), 'mem0': _w((lambda *s: _rng.normal(s) * 0.2)(B, M, Dm)), 'Wq': _w((lambda *s: _rng.normal(s) * 1.6)(Dm, H, Dh) * Dm ** (-0.5)), 'Wk': _w((lambda *s: _rng.normal(s) * 1.6)(Dm, H, Dh) * Dm ** (-0.5)), 'Wv': _w((lambda *s: _rng.normal(s) * 0.2)(Dm, H, Dh) * Dm ** (-0.5)), 'Wo': _w((lambda *s: _rng.normal(s) * 0.2)(H, Dh, Dm) * (H * Dh) ** (-0.5)), 'seg_len': seg}
    _A_in = _A_setup()

    def _B_setup():
        B, S, D, F = (1, 2048, 448, 1792)
        return {'x': _w((lambda *s: _rng.normal(s) * 0.05)(B, S, D)), 'w1': _w((lambda *s: _rng.normal(s) * 0.2)(S, F) * S ** (-0.5)), 'b1': _w((lambda *s: _rng.normal(s) * 0.2)(F) * 0.02), 'w2': _w((lambda *s: _rng.normal(s) * 0.2)(F, S) * F ** (-0.5)), 'b2': _w((lambda *s: _rng.normal(s) * 0.05)(S) * 0.02)}
    _B_in = _B_setup()
    return {'A_x': _A_in['x'], 'A_mem0': _A_in['mem0'], 'A_Wq': _A_in['Wq'], 'A_Wk': _A_in['Wk'], 'A_Wv': _A_in['Wv'], 'A_Wo': _A_in['Wo'], 'A_seg_len': _A_in['seg_len'], 'B_x': _B_in['x'], 'B_w1': _B_in['w1'], 'B_b1': _B_in['b1'], 'B_w2': _B_in['w2'], 'B_b2': _B_in['b2']}

def reference(A_x, A_mem0, A_Wq, A_Wk, A_Wv, A_Wo, A_seg_len, B_x, B_w1, B_b1, B_w2, B_b2):

    def _A_ref(x, mem0, Wq, Wk, Wv, Wo, seg_len):
        B, S, Dm = x.shape
        H, Dh = (Wq.shape[1], Wq.shape[2])
        M = mem0.shape[1]
        scale = Dh ** (-0.5)
        n_seg = S // seg_len
        L = M + seg_len
        idx = jnp.arange(L)
        mask = (idx[:, None] < M) | (idx[:, None] >= idx[None, :])
        mem = mem0
        outs = []
        for s in range(n_seg):
            xs = x[:, s * seg_len:(s + 1) * seg_len, :].copy()
            h = jnp.concatenate([mem, xs], axis=1)
            q = jnp.einsum('btd,dhe->bhte', h, Wq)
            k = jnp.einsum('btd,dhe->bhte', h, Wk)
            v = jnp.einsum('btd,dhe->bhte', h, Wv)
            scores = jnp.einsum('bhqe,bhke->bhqk', q, k) * scale
            scores = jnp.where(mask[None, None], scores, -1000000000.0)
            p = _softmax(scores, axis=-1)
            o = jnp.einsum('bhqk,bhke->bhqe', p, v)
            o = jnp.einsum('bhte,hed->btd', o, Wo)
            mem = o[:, :M, :].copy()
            outs.append(o[:, M:, :])
        return jnp.concatenate(outs, axis=1)

    def _B_ref(x, w1, b1, w2, b2):
        B, S, D = x.shape
        h = _layernorm(x, axis=-1)
        u = jnp.einsum('bsd,sf->bdf', h, w1) + b1
        u = _gelu(u)
        y = jnp.einsum('bdf,fs->bds', u, w2) + b2
        return (lambda x, *d: x.transpose(*d))(y, 0, 2, 1)
    x = A_x
    h = x + _A_ref(_layernorm(x, axis=-1), A_mem0, A_Wq, A_Wk, A_Wv, A_Wo, A_seg_len)
    h2 = h + _B_ref(_layernorm(h, axis=-1), B_w1, B_b1, B_w2, B_b2)
    return h2
```

```python
import functools
import math
import jax
import jax.numpy as jnp
from jax import lax
import jax.experimental.pallas as pl
import jax.experimental.pallas.tpu as pltpu

F32, BF16, U32 = jnp.float32, jnp.bfloat16, jnp.uint32
EPS = 1e-5
NT = (((1,), (1,)), ((), ()))


def _dot(a, b):
    return jnp.dot(a, b, preferred_element_type=F32)


def _dot_nt(a, b):
    return lax.dot_general(a, b, NT, preferred_element_type=F32)


def _ln_cols(x):
    n = x.shape[0]
    m = jnp.sum(x, axis=0, keepdims=True) * (1.0 / n)
    c = x - m
    v = jnp.sum(c * c, axis=0, keepdims=True) * (1.0 / n)
    return c * lax.rsqrt(v + EPS)


def _split_pair(u):
    lo = pltpu.bitcast(u << 16, F32).astype(BF16)
    hi = pltpu.bitcast(u & jnp.uint32(0xFFFF0000), F32).astype(BF16)
    return lo, hi


def make_kernel(S, D, H, E, M, SEG, F, cfg):
    NP = H // 2
    DM = (D // 128) * 128
    L = M + SEG
    NT_ = L // 8
    PW = 2 * DM + 128
    BLK = cfg.get("blk", 4)
    TB = BLK * SEG
    scale = (E ** -0.5) * math.log2(math.e)

    def kernel(xT_h, mem_h, wq_h, wk_h, wv_h, woT_h, w1_h, b1_h, w2_h, b2_h, out_h,
               xT_s, mem_s, wq_s, wk_s, wv_s, wo_s, w1_s, b1_s, w2_s, b2_s,
               WK, WV, Z, KT, VT, O, hT, hh, g_s, out_s,
               sem_q, sem_k, sem_v, sem_o, sem_m, sem_out):
        wq_u, wk_u, wv_u = (r.bitcast(U32) for r in (wq_h, wk_h, wv_h))
        cp_v = [pltpu.make_async_copy(wv_u.at[:, p, :], wv_s.at[p], sem_v.at[p]) for p in range(NP)]
        cp_o = [pltpu.make_async_copy(woT_h.at[pl.ds(2 * p, 2)], wo_s.at[pl.ds(2 * p, 2)], sem_o.at[p]) for p in range(NP)]
        cp_q = [pltpu.make_async_copy(wq_u.at[:, p, :], wq_s.at[p], sem_q.at[p]) for p in range(NP)]
        cp_k = [pltpu.make_async_copy(wk_u.at[:, p, :], wk_s.at[p], sem_k.at[p]) for p in range(NP)]
        cp_x = pltpu.make_async_copy(xT_h, xT_s, sem_m.at[0])
        cp_mem = pltpu.make_async_copy(mem_h, mem_s, sem_m.at[1])
        cp_w1 = pltpu.make_async_copy(w1_h, w1_s, sem_m.at[2])
        cp_w2 = pltpu.make_async_copy(w2_h, w2_s, sem_m.at[3])
        cp_b1 = pltpu.make_async_copy(b1_h, b1_s, sem_m.at[4])
        cp_b2 = pltpu.make_async_copy(b2_h, b2_s, sem_m.at[5])
        for p in range(NP):
            cp_v[p].start()
            cp_o[p].start()
        cp_x.start()
        for p in range(NP):
            cp_q[p].start()
            cp_k[p].start()
        cp_mem.start()
        cp_b1.start()
        cp_b2.start()
        cp_w1.start()
        cp_w2.start()

        lane = lax.broadcasted_iota(jnp.int32, (8, 128), 1)
        lo_half = lane < 64

        def fold(dst, p, l0, l1, r0, r1, mul):
            y0 = _dot_nt(l0, r0[:DM])
            y1 = _dot_nt(l1, r1[:DM])
            tail = jnp.concatenate([r0[DM:], r1[DM:]], axis=0)
            t0 = _dot_nt(l0, tail)
            t1 = _dot_nt(l1, tail)
            ln = lax.broadcasted_iota(jnp.int32, t0.shape, 1)
            t = jnp.where(ln < 64, t0, t1)
            y = jnp.concatenate([y0, y1, t], axis=1)
            if mul != 1.0:
                y = y * mul
            dst[:, p * PW:(p + 1) * PW] = pltpu.bitcast(y.astype(BF16), U32)

        with jax.named_scope("fold_v"):
            for p in range(NP):
                cp_v[p].wait()
                cp_o[p].wait()
                v0, v1 = _split_pair(wv_s[p])
                fold(WV, p, v0, v1, wo_s[2 * p], wo_s[2 * p + 1], 1.0)

        cp_x.wait()
        with jax.named_scope("ln_x"):
            for b in range(S // 128):
                z = _ln_cols(xT_s[:, b * 128:(b + 1) * 128].astype(F32))
                z = z.astype(BF16).astype(F32)
                z = jnp.concatenate([z, z[DM:]], axis=0)
                Z[b * 128:(b + 1) * 128, :] = z.T

        with jax.named_scope("fold_k"):
            for p in range(NP):
                cp_q[p].wait()
                cp_k[p].wait()
                q0, q1 = _split_pair(wq_s[p])
                k0, k1 = _split_pair(wk_s[p])
                fold(WK, p, k0, k1, q0, q1, scale)

        cp_mem.wait()
        mem0 = mem_s[...].astype(F32)
        mem0 = jnp.concatenate([mem0, mem0[:, DM:]], axis=1)

        row = lax.broadcasted_iota(jnp.int32, (8, 128), 0)
        tri = row >= (lane & 7)

        def project(zs, W, T, p):
            w = pltpu.bitcast(W[:, p * PW:(p + 1) * PW], BF16)
            y = _dot(zs[:, :D], w)
            for t in range(NT_):
                yt = y[8 * t:8 * t + 8]
                tail = yt[:, 2 * DM:]
                top = jnp.concatenate([yt[:, :DM], jnp.where(lo_half, tail, 0.0)], axis=1)
                bot = jnp.concatenate([yt[:, DM:2 * DM], jnp.where(lo_half, 0.0, tail)], axis=1)
                blk = jnp.concatenate([top, bot], axis=0).astype(BF16)
                r0 = (t * 128 + 16 * p) // 2
                T[r0:r0 + 8, :] = pltpu.bitcast(blk, U32)

        def allreduce8(x, op):
            for k in (1, 2, 4):
                y = jnp.where((lane & k) != 0, pltpu.roll(x, k, 1), pltpu.roll(x, 128 - k, 1))
                x = op(x, y)
            return x

        def softmax(s):
            rows = []
            for r in range(NT_):
                tiles = [s[8 * r:8 * r + 8, 128 * t:128 * t + 128] for t in range(NT_)]
                if r > 0:
                    tiles[r] = jnp.where(tri, tiles[r], -1e9)
                    tiles = tiles[:r + 1]
                m = functools.reduce(jnp.maximum, tiles)
                m = allreduce8(m, jnp.maximum)
                e = [jnp.exp2(x - m) for x in tiles]
                l = allreduce8(functools.reduce(jnp.add, e), jnp.add)
                inv = 1.0 / l
                pr = [x * inv for x in e]
                pr += [jnp.zeros((8, 128), F32)] * (NT_ - len(pr))
                rows.append(jnp.concatenate(pr, axis=1))
            return jnp.concatenate(rows, axis=0)

        def step(mem, t0):
            zs = jnp.concatenate([mem, Z[pl.ds(t0, SEG), :]], axis=0)
            for p in range(NP):
                project(zs, WK, KT, p)
            project(zs, WV, VT, 0)
            s = _dot_nt(zs, pltpu.bitcast(KT[...], BF16))
            pr = softmax(s)
            for p in range(1, NP):
                project(zs, WV, VT, p)
            o = _dot(pr, pltpu.bitcast(VT[...], BF16))
            tail = o[:, DM:]
            tail = tail + pltpu.roll(tail, 64, 1)
            o = jnp.concatenate([o[:, :DM], tail], axis=1)
            return o[:M], o[M:]

        def body(b, mem):
            base = pl.multiple_of(b * TB, TB)
            for j in range(BLK):
                mem, o = step(mem, pl.multiple_of(base + j * SEG, SEG))
                O[pl.ds(pl.multiple_of(base + j * SEG, SEG), SEG), :] = o
            return mem

        with jax.named_scope("recur"):
            lax.fori_loop(0, S // TB, body, mem0)

        with jax.named_scope("resid_ln"):
            for b in range(S // 128):
                cs = slice(b * 128, (b + 1) * 128)
                h = O[cs, :].T[:D] + xT_s[:, cs].astype(F32)
                hT[:, cs] = h
                hh[:, cs] = _ln_cols(_ln_cols(h)).astype(BF16)

        cp_b1.wait()
        cp_b2.wait()
        cp_w1.wait()
        b1 = b1_s[...].astype(F32)
        b2 = b2_s[...].astype(F32)
        FC = cfg.get("fc", 256)
        with jax.named_scope("mix1"):
            for f0 in range(0, F, FC):
                u = _dot(hh[...], w1_s[:, f0:f0 + FC])
                bias = jnp.concatenate([b1[r:r + 1] for r in range(f0 // 128, (f0 + FC) // 128)], axis=1)
                g_s[:, f0:f0 + FC] = jax.nn.gelu(u + bias, approximate=True).astype(BF16)
        cp_w2.wait()
        SC = cfg.get("sc", 256)
        cps = []
        with jax.named_scope("mix2"):
            for i, s0 in enumerate(range(0, S, SC)):
                y = _dot(g_s[...], w2_s[:, s0:s0 + SC])
                bias = jnp.concatenate([b2[r:r + 1] for r in range(s0 // 128, (s0 + SC) // 128)], axis=1)
                out_s[:, s0:s0 + SC] = (y + bias + hT[:, s0:s0 + SC]).astype(BF16)
                cp = pltpu.make_async_copy(out_s.at[:, pl.ds(s0, SC)], out_h.at[:, pl.ds(s0, SC)], sem_out.at[i])
                cp.start()
                cps.append(cp)
        for cp in cps:
            cp.wait()

    return kernel


def build(cfg):
    def fn(A_x, A_mem0, A_Wq, A_Wk, A_Wv, A_Wo, A_seg_len, B_x, B_w1, B_b1, B_w2, B_b2):
        _, S, D = A_x.shape
        M = A_mem0.shape[1]
        H, E = A_Wq.shape[1:]
        F = B_w1.shape[1]
        SEG = 32
        NP = H // 2
        DP = -(-D // 128) * 128
        NW = NP * (2 * (D // 128) * 128 + 128)
        LT = (M + SEG) // 8 * 128
        SC = cfg.get("sc", 256)
        any_spec = pl.BlockSpec(memory_space=pl.ANY)
        V = pltpu.VMEM
        outT = pl.pallas_call(
            make_kernel(S, D, H, E, M, SEG, F, cfg),
            in_specs=[any_spec] * 10,
            out_specs=any_spec,
            out_shape=jax.ShapeDtypeStruct((D, S), A_x.dtype),
            scratch_shapes=[
                V((D, S), BF16), V((M, D), BF16),
                V((NP, D, E), U32), V((NP, D, E), U32), V((NP, D, E), U32), V((H, D, E), BF16),
                V((S, F), BF16), V((F // 128, 128), BF16), V((F, S), BF16), V((S // 128, 128), BF16),
                V((D // 2, NW), U32), V((D // 2, NW), U32), V((S, DP), F32),
                V((LT // 2, DP), U32), V((LT // 2, DP), U32), V((S, DP), F32),
                V((D, S), F32), V((D, S), BF16), V((D, F), BF16), V((D, S), BF16),
                pltpu.SemaphoreType.DMA((NP,)), pltpu.SemaphoreType.DMA((NP,)),
                pltpu.SemaphoreType.DMA((NP,)), pltpu.SemaphoreType.DMA((NP,)),
                pltpu.SemaphoreType.DMA((6,)), pltpu.SemaphoreType.DMA((S // SC,)),
            ],
            compiler_params=pltpu.CompilerParams(vmem_limit_bytes=110 * 1024 * 1024, flags=cfg.get("flags")),
        )(jnp.swapaxes(A_x[0], 0, 1), A_mem0[0], A_Wq, A_Wk, A_Wv, jnp.swapaxes(A_Wo, 1, 2),
          B_w1, B_b1.reshape(F // 128, 128), B_w2, B_b2.reshape(S // 128, 128))
        return jnp.swapaxes(outT, 0, 1)[None]
    return fn


@jax.jit
def pallas_sequential_preLN__memory_aug_recurrent_mem_tr__mixer_token_mlp__prompt_kernel(
    A_x, A_mem0, A_Wq, A_Wk, A_Wv, A_Wo, A_seg_len, B_x, B_w1, B_b1, B_w2, B_b2,
):
    return build({})(A_x, A_mem0, A_Wq, A_Wk, A_Wv, A_Wo, A_seg_len, B_x, B_w1, B_b1, B_w2, B_b2)
```

```python
import functools
import math
import jax
import jax.numpy as jnp
from jax import lax
import jax.experimental.pallas as pl
import jax.experimental.pallas.tpu as pltpu

F32, BF16, U32 = jnp.float32, jnp.bfloat16, jnp.uint32
EPS = 1e-5

_dot = functools.partial(jnp.dot, preferred_element_type=F32)
_dot_nt = functools.partial(lax.dot_general, dimension_numbers=(((1,), (1,)), ((), ())),
                            preferred_element_type=F32)


def _split_pair(u):
    lo = pltpu.bitcast(u << 16, F32).astype(BF16)
    hi = pltpu.bitcast(u & jnp.uint32(0xFFFF0000), F32).astype(BF16)
    return lo, hi


def _pack(x):
    return pltpu.bitcast(x.astype(BF16), U32)


def _pack2(a, b):
    return pltpu.pack_elementwise([a, b], packed_dtype=BF16)


def _unpack(u):
    return pltpu.bitcast(u, BF16)


_HK_STEP = (
    (((1, 0, 0), (0, 0, 0)), ((1, 0, -1), (-1, 0, 0), (0, 0, 0)), ((1, 0, 0), (-1, 0, 0))),
    (((0, 1, 0), (0, 1, 0)), ((0, 0, 0), (-1, 1, 0), (0, -1, 0)), ((0, 1, 0), (0, 0, 0))),
    (((0, 0, 1), (0, 0, 0)), ((0, 0, 0), (0, 0, -1), (-1, 0, 1)), ((0, 0, 1), (0, 0, 0))),
    (((1, 1, 0), (0, 0, 0)), ((0, 0, 0), (1, 0, 0), (0, 0, 0)), ((1, 1, 0), (0, 0, 0))),
    (((1, 0, 0), (0, -1, 0)), ((0, 1, 0), (-1, 0, 0), (0, 0, 0)), ((0, 1, 0), (1, 0, 0))),
    (((1, 0, 1), (1, 0, 1)), ((0, 0, 0), (0, 0, 0), (1, 0, 0)), ((1, 0, 1), (0, 0, 0))),
    (((1, 0, 0), (1, 0, 1)), ((0, 0, 1), (0, 0, 0), (-1, 0, 0)), ((1, 0, 1), (-1, 0, 0))),
    (((0, 1, 1), (0, 0, 0)), ((0, 0, 0), (0, 0, 1), (0, 0, 0)), ((0, 1, 1), (0, -1, -1))),
    (((0, 1, 1), (0, 1, 0)), ((0, 0, 0), (0, 0, -1), (0, 1, 0)), ((0, 1, 0), (0, -1, -1))),
)
_HK_AHEAD = (
    (((1, 0, 0), (1, 0, 0)), ((1, -1, 0), (0, 0, 0), (-1, 0, 0)), ((0, 0, 0), (1, 0, 0))),
    (((0, 0, 0), (0, 1, 0)), ((0, 1, 0), (0, -1, 1), (0, 0, 0)), ((0, 1, 0), (0, -1, 0))),
    (((0, 0, 0), (0, 0, 1)), ((0, 0, -1), (0, 0, 0), (0, -1, 1)), ((0, 0, 0), (0, 0, 1))),
    (((0, 0, 0), (1, 1, 0)), ((0, 1, 0), (0, 0, 0), (0, 0, 0)), ((0, 0, 0), (1, 1, 0))),
    (((0, 0, 0), (1, 0, 1)), ((0, 0, -1), (0, 0, 0), (0, 0, 0)), ((1, 0, 1), (-1, 0, -1))),
    (((0, 1, 1), (0, 1, 1)), ((0, 0, 0), (0, 0, 0), (0, 1, 0)), ((0, 0, 0), (0, 1, 1))),
)
_HK_MIX = sorted({tuple(o[g][c] for _, _, o in _HK_AHEAD) for g in range(2) for c in range(3)}, reverse=True)
_HK_MIX_OF = [[_HK_MIX.index(tuple(o[g][c] for _, _, o in _HK_AHEAD)) for c in range(3)] for g in range(2)]


def _signed_sum(coefs, values):
    terms = sorted(((c, i) for i, c in enumerate(coefs) if c), key=lambda t: -t[0])
    acc = values[terms[0][1]] if terms[0][0] > 0 else -values[terms[0][1]]
    for c, i in terms[1:]:
        acc = acc + values[i] if c > 0 else acc - values[i]
    return acc


def _flat(rows):
    return [c for row in rows for c in row]


def _tiles(ref, start, count, axis):
    return _unpack(jnp.concatenate([ref[start + i] for i in range(count)], axis=axis))


def _strassen_lhs(a11, a12, a21, a22):
    return [a11 + a22, a21 + a22, a11, a22, a11 + a12, a21 - a11, a12 - a22]


def _strassen_rhs(b11, b12, b21, b22):
    return [b11 + b22, b11, b12 - b22, b21 - b11, b22, b11 + b12, b21 + b22]


def _strassen_out(m1, m2, m3, m4, m5, m6, m7):
    return m1 + m4 - m5 + m7, m3 + m5, m2 + m4, m1 - m2 + m3 + m6


def _packed_rhs(quads):
    lo = _strassen_rhs(*[pltpu.bitcast(q << 16, F32) for q in quads])
    hi = _strassen_rhs(*[pltpu.bitcast(q & jnp.uint32(0xFFFF0000), F32) for q in quads])
    out = [_pack2(a, b) for a, b in zip(lo, hi)]
    out[1], out[4] = quads[0], quads[3]
    return out


ORDER = ("H H H H H kt t3 km:02 !H G km:24 !t3 km:46 !G km:68 t0 t1 t2 q vt d s vm:07 f vm:78 "
         "Z Z Z T N X g !Z h !T !N !X b")
ORDER0 = ORDER.replace("Z Z Z T N X g !Z h !T !N !X b", "T N g h !T !N x")


def make_kernel(S, D, H, E, M, SEG, F, cfg):
    NP = H // 2
    NC = D // 128
    DM = NC * 128
    L = M + SEG
    G = L // 8
    TB = 128
    SPB = TB // SEG
    BLK = cfg.get("blk", 2)
    NB = S // TB
    NS = S // SEG
    scale = (E ** -0.5) * math.log2(math.e)
    NCH = cfg.get("nch", 512)
    ZL = 16
    XL = ZL // SPB + 1
    LOOK = cfg.get("look", 2)

    def kernel(xT_h, mem_h, wq_h, wk_h, wv_h, woT_h, w1_h, b1_h, w2_h, b2_h, out_h,
               xT_s, mem_s, wq_s, wk_s, wv_s, wo_s, w1_s, b1_s, w2_s, b2_s,
               WK, WV, WA, TK, TV, AH, WQ2, B2, X, Z, KT, KX, GX, VT, O, HS, NS_, hT, nT, U, GA, out_s,
               sem_q, sem_k, sem_v, sem_o, sem_m, sem_out):
        wq_u, wk_u, wv_u = (r.bitcast(U32) for r in (wq_h, wk_h, wv_h))
        def v_copies(p):
            return [pltpu.make_async_copy(wv_u.at[:, p, :], wv_s.at[p], sem_v.at[p]),
                    pltpu.make_async_copy(woT_h.at[pl.ds(2 * p, 2)], wo_s.at[pl.ds(2 * p, 2)], sem_o.at[p])]

        def k_copies(p):
            return [pltpu.make_async_copy(wq_u.at[:, p, :], wq_s.at[p], sem_q.at[p]),
                    pltpu.make_async_copy(wk_u.at[:, p, :], wk_s.at[p], sem_k.at[p])]

        cp_x0 = pltpu.make_async_copy(xT_h.at[:, pl.ds(0, XL * TB)], xT_s.at[:, pl.ds(0, XL * TB)], sem_m.at[0])
        cp_x1 = pltpu.make_async_copy(xT_h.at[:, pl.ds(XL * TB, S - XL * TB)], xT_s.at[:, pl.ds(XL * TB, S - XL * TB)], sem_m.at[1])
        cp_mem = pltpu.make_async_copy(mem_h, mem_s, sem_m.at[2])
        cp_w1 = pltpu.make_async_copy(w1_h, w1_s, sem_m.at[3])
        cp_w2 = pltpu.make_async_copy(w2_h, w2_s, sem_m.at[4])
        cp_b1 = pltpu.make_async_copy(b1_h, b1_s, sem_m.at[5])
        cp_b2 = pltpu.make_async_copy(b2_h, b2_s, sem_m.at[6])
        small = [cp_x0, cp_mem, cp_b1, cp_b2]
        mode0 = cfg.get("dma", 0)
        if mode0 == 0:
            for cp in small:
                cp.start()
        for p in range(NP):
            for cp in v_copies(p):
                cp.start()
            if mode0 == p + 1:
                for cp in small:
                    cp.start()
        for p in range(NP):
            for cp in k_copies(p):
                cp.start()
        cp_x1.start()

        lane = lax.broadcasted_iota(jnp.int32, (8, 128), 1)
        lo_half = lane < 64

        def lo_mask(n):
            return lax.broadcasted_iota(jnp.int32, (n, 128), 1) < 64

        def store_main(W, y, h, side):
            blocks = [y[128 * k:128 * k + 128, 128 * c:128 * c + 128] for k in range(NC) for c in range(NC)]
            for r, (_, coefs, _) in enumerate(_HK_STEP):
                W[r, h] = _pack(_signed_sum(_flat(coefs), blocks))
            for r, (_, coefs, _) in enumerate(_HK_AHEAD):
                WA[r, side * H + h] = _pack(_signed_sum(_flat(coefs), blocks))

        def ahead(sb, hs, count, after=lambda v: v):
            base = pl.multiple_of(sb * 8 * SEG, 8 * SEG)
            x = [jnp.concatenate([Z[k, pl.ds(base + n * SEG + SEG - 16 + 8 * g, 8), :] for n in range(8)], axis=0)
                 for g in range(2) for k in range(NC)]
            m = [_dot(after(_signed_sum(_flat(coefs), x)), _tiles(WA.at[r], hs, count, 1))
                 for r, (coefs, _, _) in enumerate(_HK_AHEAD)]
            for n, coefs in enumerate(_HK_MIX):
                v = _signed_sum(coefs, m)
                for i in range(count):
                    AH[sb & 1, hs + i, n] = v[:, 128 * i:128 * i + 128]

        def x_piece(src, dst, j):
            r0 = pl.multiple_of(j * 128, 64)
            r1 = pl.multiple_of(jnp.minimum(j * 128 + 64, DM), 64)
            t = jnp.concatenate([xT_s[pl.ds(r0, 64), pl.ds(src, TB)], xT_s[pl.ds(r1, 64), pl.ds(src, TB)]], axis=0)
            X[j, pl.ds(dst, TB), :] = t.astype(F32).T

        def layernorm(tiles):
            mask = lo_mask(tiles[0].shape[0])

            def mean(ts):
                acc = functools.reduce(jnp.add, ts[:NC]) + jnp.where(mask, ts[NC], 0.0)
                return jnp.sum(acc, axis=1, keepdims=True) * (1.0 / D)

            m = mean(tiles)
            yield
            c = [t - m for t in tiles]
            v = mean([t * t for t in c])
            yield
            r = lax.rsqrt(v + EPS)
            return [t * r for t in c]

        def z_piece(src, dst, rows=SEG):
            z = yield from layernorm([X[c, pl.ds(src, rows), :] for c in range(NC + 1)])
            for c in range(NC + 1):
                Z[c, pl.ds(dst, rows), :] = z[c]

        def h_piece(t0, slot, dst_slot, dst):
            h = [X[c, pl.ds(t0, SEG), :] + O[slot, c] for c in range(NC + 1)]
            for c in range(NC + 1):
                HS[dst_slot, c, pl.ds(dst, SEG), :] = h[c]
            n = yield from layernorm(h)
            n = yield from layernorm(n)
            for c in range(NC + 1):
                NS_[dst_slot, c, pl.ds(dst, SEG), :] = n[c]

        def finish(gen):
            for _ in gen:
                pass

        def ht_piece(slot, col, j):
            hT[pl.ds(pl.multiple_of(j * 128, 128), 128), pl.ds(col, TB)] = HS[slot, j].T

        def nt_piece(slot, col, j):
            nT[pl.ds(pl.multiple_of(j * 128, 128), 128), pl.ds(col, TB)] = NS_[slot, j].T

        O[...] = jnp.zeros(O.shape, F32)
        HS[1] = jnp.zeros(HS.shape[1:], F32)
        NS_[...] = jnp.zeros(NS_.shape, F32)
        hT[0:TB, 0:128] = jnp.zeros((TB, 128), F32)
        nT[0:TB, 0:128] = jnp.zeros((TB, 128), F32)

        def setup():
            for cp in small:
                cp.wait()
            for b in range(XL):
                for j in range(NC + 1):
                    x_piece(b * TB, b * TB, j)
            for b in range(ZL // SPB):
                finish(z_piece(b * TB, b * TB, TB))
            b1 = b1_s[...].astype(F32)
            for r in range(F // 128):
                U[:, r * 128:(r + 1) * 128] = jnp.broadcast_to(b1[r:r + 1], (D, 128))

        if mode0 == 0:
            setup()

        def tail_first(w):
            return jnp.concatenate([w[DM:], w[:DM]], axis=0)

        def fold_v(p, _):
            if mode0:
                pl.when(p == mode0)(setup)
            for cp in v_copies(p):
                cp.wait()
            v0, v1 = _split_pair(wv_s[p])
            o0, o1 = wo_s[2 * p], wo_s[2 * p + 1]
            t = jnp.concatenate([_dot_nt(o0[DM:], v0), _dot_nt(o1[DM:], v1)], axis=0)
            t = jnp.concatenate([t, jnp.zeros((128, 64), F32)], axis=1).T
            TV[p] = _pack(t[:DM])
            y0, y1 = _dot_nt(tail_first(v0), o0[:DM]), _dot_nt(tail_first(v1), o1[:DM])
            store_main(WV, y0[64:], 2 * p, 1)
            store_main(WV, y1[64:], 2 * p + 1, 1)
            m = lo_mask(64)
            top = jnp.concatenate([y0[:64], jnp.where(m, t[DM:D], 0.0)], axis=1)
            bot = jnp.concatenate([y1[:64], jnp.where(m, 0.0, t[DM:D])], axis=1)
            B2[p] = _pack(jnp.concatenate([top, bot], axis=0))

        def fold_k(p, _):
            for cp in k_copies(p):
                cp.wait()
            ahead(0, H + 2 * p, 2)
            q0, q1 = _split_pair(wq_s[p])
            k0, k1 = _split_pair(wk_s[p])
            t = jnp.concatenate([_dot_nt(q0[DM:], k0), _dot_nt(q1[DM:], k1)], axis=0) * scale
            t = jnp.concatenate([t, jnp.zeros((128, 64), F32)], axis=1)
            TK[p] = _pack(t[:, :DM].T)
            corner = t[:64, DM:] + pltpu.roll(t[64:, DM:], 64, 1)
            WQ2[p, DM // 2:, :] = _pack(corner)
            y0 = _dot_nt(tail_first(k0), q0[:DM]) * scale
            y1 = _dot_nt(tail_first(k1), q1[:DM]) * scale
            store_main(WK, y0[64:], 2 * p, 0)
            store_main(WK, y1[64:], 2 * p + 1, 0)
            q2 = jnp.concatenate([y0[:64], y1[:64]], axis=0).T
            WQ2[p, :DM // 2, :] = _pack(q2)

        with jax.named_scope("fold_v"):
            lax.fori_loop(0, NP, fold_v, None)
        with jax.named_scope("fold_k"):
            lax.fori_loop(0, NP, fold_k, None)

        for cp in (cp_w1, cp_w2):
            cp.start()
        with jax.named_scope("ahead0"):
            for hs in range(0, H, 4):
                ahead(0, hs, 4)
        cp_x1.wait()
        mem0 = mem_s[...].astype(F32)
        mem0 = jnp.concatenate([mem0, mem0[:, DM:]], axis=1)

        row = lax.broadcasted_iota(jnp.int32, (8, 128), 0)
        tri = row >= ((lane >> 1) & 7)
        blockid = lane >> 4

        def project_tail(z1, W, T, after):
            for p0 in range(0, NP, 4):
                y = _dot(after(z1), _tiles(W, p0, 4, 1))
                for t in range(G):
                    for i in range(4):
                        v = y[8 * t:8 * t + 8, 128 * i:128 * i + 128]
                        r0 = t * 64 + 8 * (p0 + i)
                        T[NC, r0:r0 + 8, :] = _pack2(jnp.where(lo_half, v, 0.0), jnp.where(lo_half, 0.0, v))

        HC = cfg.get("hc", 2)

        def project_main(lhs, W, T, side, early, after, lo, hi):
            for h0 in range(2 * lo, 2 * hi, HC):
                m = [_dot(after(a), _tiles(W.at[r], h0, HC, 1)) for r, a in enumerate(lhs)]
                last = [v[L - 16:] for v in m]
                for c in range(NC):
                    y = _signed_sum([o[0][c] for _, _, o in _HK_STEP], m)
                    u = _signed_sum([o[1][c] for _, _, o in _HK_STEP], last)
                    for i in range(0, HC, 2):
                        rows = []
                        for k in (i, i + 1):
                            cs = slice(128 * k, 128 * k + 128)
                            hs = side * H + h0 + k
                            rows.append([y[8 * t:8 * t + 8, cs] for t in range(G - 2)]
                                        + [y[L - 16:, cs] + early(hs, _HK_MIX_OF[0][c]),
                                           u[:, cs] + early(hs, _HK_MIX_OF[1][c])])
                        for t in range(G):
                            r0 = t * 64 + 4 * (h0 + i)
                            T[c, r0:r0 + 8, :] = _pack2(rows[0][t], rows[1][t])

        def allreduce8(x, op):
            for k in (2, 4, 8):
                y = jnp.where((lane & k) != 0, pltpu.roll(x, k, 1), pltpu.roll(x, 128 - k, 1))
                x = op(x, y)
            return x

        def groups(t):
            if cfg.get("full"):
                return list(range(G))
            return [0] + list(range(max(min(t, cfg.get("tmax", 9)), 1), G))

        def ntiles(r):
            return G if r == 0 else r + 1

        def step(mem, s, side, probes, keep, order):
            t0 = pl.multiple_of(s * SEG, SEG)
            zt = [jnp.concatenate([mem[:, 128 * c:128 * c + 128], Z[c, pl.ds(t0, SEG), :]], axis=0) for c in range(NC + 1)]
            full = [v[:L - 8] for v in zt[:NC]]
            pair = [v[L - 16:L - 8] for v in zt[:NC]] + [v[L - 8:] for v in zt[:NC]]
            lhs = [jnp.concatenate([_signed_sum(coefs[0], [v[:L - 16] for v in full]), _signed_sum(_flat(coefs), pair)], axis=0)
                   for coefs, _, _ in _HK_STEP]
            early = lambda hs, n: AH[(s >> 3) & 1, hs, n, pl.ds(pl.multiple_of((s & 7) * 8, 8), 8), :]
            zs = jnp.concatenate(zt, axis=1)
            z1 = zs[:, :DM]
            z2 = zt[NC]
            g = [_pack2(jnp.where(lo_half, z2[8 * t:8 * t + 8], 0.0),
                        jnp.where(lo_half, 0.0, z2[8 * t:8 * t + 8])) for t in range(G)]
            zero = jnp.zeros((8, 128), g[0].dtype)
            Gp = [_unpack(jnp.concatenate([g[(b - p) % NP] if (b - p) % NP < G else zero for b in range(NP)], axis=0))
                  for p in range(NP)]
            st = {"wait": []}

            def after(lhs):
                if not st["wait"]:
                    return lhs
                head = lhs[:8, :128]
                for v in st["wait"]:
                    head = jnp.where(keep, head, v)
                st["wait"] = []
                if lhs.shape[1] > 128:
                    head = jnp.concatenate([head, lhs[:8, 128:]], axis=1)
                return jnp.concatenate([head, lhs[8:]], axis=0)

            def q2_proj():
                st["q2"] = _dot(after(zs[:, :D]), _tiles(WQ2, 0, NP, 1))

            mode = cfg.get("gx", "roll")

            def g_transpose():
                if mode == "nt":
                    return
                g0 = pltpu.bitcast(Gp[0].T, U32)
                for p in range(NP):
                    if mode == "roll":
                        GX[p] = pltpu.roll(g0, 16 * p, 1) if p else g0
                    else:
                        GX[p] = pltpu.bitcast(Gp[p].T, U32)

            def term2():
                q2 = st["q2"]
                if mode == "nt":
                    o = [_dot_nt(q2[:, 128 * p:128 * p + 128], Gp[p]) for p in range(NP)]
                else:
                    o = [_dot(after(q2[:, 128 * p:128 * p + 128]), _unpack(GX[p])) for p in range(NP)]
                extra = []
                for r in range(G):
                    rowt = []
                    for t in range(ntiles(r)):
                        x = o[0][8 * r:8 * r + 8]
                        for p in range(1, NP):
                            x = jnp.where(blockid == (p + t) % NP, o[p][8 * r:8 * r + 8], x)
                        rowt.append(pltpu.roll(x, 128 - 16 * t, 1) if t else x)
                    extra.append(rowt)
                st["extra"] = extra

            def k_transpose(c):
                KX[c] = pltpu.bitcast(_unpack(KT[c]).T, U32)

            def scores():
                s = {}
                for t in range(G):
                    rs = groups(t)
                    lhs = after(jnp.concatenate([zs[8 * r:8 * r + 8] for r in rs], axis=0))
                    rhs = jnp.concatenate([_unpack(KX[c, :, 128 * t:128 * t + 128]) for c in range(NC + 1)], axis=0)
                    y = _dot(lhs, rhs)
                    for i, r in enumerate(rs):
                        s[r, t] = y[8 * i:8 * i + 8]
                pt = []
                for r in range(G):
                    tiles = [s[r, t] + st["extra"][r][t] for t in range(ntiles(r))]
                    if r > 0:
                        tiles[r] = jnp.where(tri, tiles[r], -1e9)
                    m = allreduce8(functools.reduce(jnp.maximum, tiles), jnp.maximum)
                    e = [jnp.exp2(x - m) for x in tiles]
                    l = allreduce8(functools.reduce(jnp.add, e), jnp.add)
                    inv = pl.reciprocal(l, approx=True)
                    inv = inv * (2.0 - l * inv)
                    for _ in range(cfg.get("pad", 0)):
                        inv = pltpu.roll(pltpu.roll(inv, 16, 1), 112, 1)
                    pt.append([x * inv for x in e])
                st["pt"] = pt

            def pz2():
                pt = st["pt"]
                sk = [[pltpu.roll(x, 16 * t, 1) if t else x for t, x in enumerate(rowt)] for rowt in pt]
                pz = []
                for p in range(NP):
                    rows = []
                    for r in range(G):
                        n = ntiles(r)
                        x = sk[r][0] if n == G else jnp.where(blockid == p, sk[r][0], 0.0)
                        for t in range(1, n):
                            x = jnp.where(blockid == (p + t) % NP, sk[r][t], x)
                        rows.append(x)
                    pz.append(_dot(after(jnp.concatenate(rows, axis=0)), Gp[p]))
                st["pz"] = jnp.concatenate(pz, axis=1)

            def b2():
                y = _dot(after(st["pz"]), _tiles(B2, 0, NP, 0))
                st["o"] = [y[8 * r:8 * r + 8] for r in range(G)]

            def pv():
                for t in range(G):
                    rs = groups(t)
                    zf = jnp.zeros((8, 128), F32)
                    lhs = after(jnp.concatenate([st["pt"][r][t] if t < ntiles(r) else zf for r in rs], axis=0))
                    rhs = jnp.concatenate([_unpack(VT[c, 64 * t:64 * t + 64, :]) for c in range(NC + 1)], axis=1)
                    y = _dot(lhs, rhs)
                    for i, r in enumerate(rs):
                        st["o"][r] = st["o"][r] + y[8 * i:8 * i + 8]

            items = {"q": q2_proj, "G": g_transpose, "d": term2, "s": scores, "f": pz2, "g": b2, "h": pv,
                     "kt": functools.partial(project_tail, z1, TK, KT, after),
                     "vt": functools.partial(project_tail, z1, TV, VT, after),
                     "km": functools.partial(project_main, lhs, WK, KT, 0, early, after),
                     "vm": functools.partial(project_main, lhs, WV, VT, 1, early, after)}
            for c in range(NC + 1):
                items[f"t{c}"] = functools.partial(k_transpose, c)
            for name in order.split():
                if name[0] == "!":
                    if name[1] == "G":
                        st["wait"].append(pltpu.bitcast(GX[NP - 1, 56:64, :], F32))
                    elif name[1] == "t":
                        c = int(name[2])
                        st["wait"].append(pltpu.bitcast(KX[c, 56:64, 128 * (G - 1):], F32))
                    else:
                        st["wait"].append(probes[name[1:]]())
                elif ":" in name:
                    items[name[:2]](int(name[3]), int(name[4]))
                elif name in side:
                    side[name](after)
                else:
                    items[name]()
            o = jnp.concatenate(st["o"], axis=0)
            tail = o[:, DM:]
            o = jnp.concatenate([o[:, :DM], tail + pltpu.roll(tail, 64, 1)], axis=1)
            return o[:M], o[M:]

        DH, FH, SH = D // 2, F // 2, S // 2

        def segment(i, s, mem, extra, order):
            b, j = s >> 2, s & 3
            col = lambda blk: pl.multiple_of(jnp.clip(blk, 0, NB - 1) * TB, TB)
            sp = s - 1
            hp = h_piece(pl.multiple_of(jnp.maximum(sp, 0) * SEG, SEG), sp & 3, (sp >> 2) & 1,
                         pl.multiple_of((sp & 3) * SEG, SEG))
            zp = z_piece(pl.multiple_of(jnp.minimum(s + ZL, NS - 1) * SEG, SEG),
                         pl.multiple_of(jnp.minimum(s + ZL, NS) * SEG, SEG))
            side = {"H": lambda a: next(hp, None), "Z": lambda a: next(zp, None),
                    "T": lambda a: ht_piece(1 - (b & 1), col(b - 1), j),
                    "N": lambda a: nt_piece(1 - (b & 1), col(b - 1), j),
                    "X": lambda a: x_piece(col(b + XL), pl.multiple_of(jnp.minimum(b + XL, NB) * TB, TB), j), **extra}
            u = (i >> 1) & 1
            rows = lambda n: pl.ds(pl.multiple_of(((i >> 2) & (n // 8 - 1)) * 8, 8), 8)
            probes = {"H": lambda: NS_[u, 0, rows(TB), :], "Z": lambda: Z[i & 3, rows(TB), :],
                      "T": lambda: hT[rows(TB), 0:128], "N": lambda: nT[rows(TB), 0:128],
                      "X": lambda: X[i & 3, rows(TB), :]}
            mem, o = step(mem, s, side, probes, lane < i + 128, order)
            for c in range(NC + 1):
                O[s & 3, c] = o[:, 128 * c:128 * c + 128]
            return mem

        S1 = NS - 8
        RC = D // SPB
        KL = (NS - S1) // SPB * TB

        def body(i, mem):
            for jj in range(2):
                s = 2 * i + jj
                extra = {"b": lambda after: ahead((s >> 3) + 1, (s & 7) * 4, 4, after)}
                mem = segment(i, s, mem, extra, cfg.get("order", ORDER))
            return mem

        def tail_body(n, mem):
            def mix(after):
                k0 = pl.multiple_of((n >> 2) * TB, TB)
                r0 = pl.multiple_of((n & 3) * RC, 8)
                U[pl.ds(r0, RC), :] += _dot(after(nT[pl.ds(r0, RC), pl.ds(k0, TB)]), w1_s[pl.ds(k0, TB), :])

            return segment(n, S1 + n, mem, {"x": mix}, cfg.get("order0", ORDER0))

        with jax.named_scope("recur"):
            mem = lax.fori_loop(0, S1 // 2, body, mem0)
        cp_w1.wait()
        with jax.named_scope("tail"):
            lax.fori_loop(0, NS - S1, tail_body, mem)
        cp_w2.wait()

        def rhs_quads(w, r0, rh, c0, ch, width):
            return _packed_rhs([pltpu.bitcast(w[r0 + dr:r0 + dr + rh, c0 + dc:c0 + dc + width], U32)
                                for dr in (0, rh) for dc in (0, ch)])

        with jax.named_scope("mix1"):
            last = (NB - 1) & 1
            KH = (S - KL) // 2
            finish(h_piece((NS - 1) * SEG, (NS - 1) & 3, last, (SPB - 1) * SEG))
            a11, a21 = nT[:DH, KL:KL + KH], nT[DH:D, KL:KL + KH]
            a3, a6 = a11.astype(BF16), (a21 - a11).astype(BF16)
            for t in range(0, FH, 128):
                w = rhs_quads(w1_s, KL, KH, t, FH, 128)
                m3 = _dot(a3, _unpack(w[2]))
                U[:DH, FH + t:FH + t + 128] += m3
                U[DH:, FH + t:FH + t + 128] += m3 + _dot(a6, _unpack(w[5]))
            for j in range(NC + 1):
                nt_piece(last, (NB - 1) * TB, j)
            for j in range(NC + 1):
                ht_piece(last, (NB - 1) * TB, j)
            a = [v.astype(BF16) for v in _strassen_lhs(a11, nT[:DH, KL + KH:], a21, nT[DH:D, KL + KH:])]
            for t in range(0, FH, 128):
                w = rhs_quads(w1_s, KL, KH, t, FH, 128)
                m1, m2, m4, m5, m7 = (_dot(a[k], _unpack(w[k])) for k in (0, 1, 3, 4, 6))
                u = (U[:DH, t:t + 128] + (m1 + m4 - m5 + m7), U[:DH, FH + t:FH + t + 128] + m5,
                     U[DH:, t:t + 128] + (m2 + m4), U[DH:, FH + t:FH + t + 128] + (m1 - m2))
                g = [jax.nn.gelu(v, approximate=True) for v in u]
                for k, v in enumerate(_strassen_lhs(*g)):
                    GA[k, :, t:t + 128] = _pack(v)
        b2v = b2_s[...].astype(F32)
        SC = cfg.get("sc", 128)
        cps = []
        with jax.named_scope("mix2"):
            for i, s0 in enumerate(range(0, SH, SC)):
                w = rhs_quads(w2_s, 0, FH, s0, SH, SC)
                m = [_dot(_unpack(GA[k]), _unpack(w[k])) for k in range(7)]
                for q, y in enumerate(_strassen_out(*m)):
                    rs = slice((q >> 1) * DH, (q >> 1) * DH + DH)
                    c0 = (q & 1) * SH + s0
                    bias = jnp.concatenate([b2v[r:r + 1] for r in range(c0 // 128, (c0 + SC) // 128)], axis=1)
                    out_s[rs, c0:c0 + SC] = (y + bias + hT[rs, c0:c0 + SC]).astype(BF16)
                for half in range(2):
                    c0 = half * SH + s0
                    cp = pltpu.make_async_copy(out_s.at[:, pl.ds(c0, SC)], out_h.at[:, pl.ds(c0, SC)],
                                               sem_out.at[2 * i + half])
                    cp.start()
                    cps.append(cp)
        for cp in cps:
            cp.wait()

    return kernel


def build(cfg):
    def fn(A_x, A_mem0, A_Wq, A_Wk, A_Wv, A_Wo, A_seg_len, B_x, B_w1, B_b1, B_w2, B_b2):
        _, S, D = A_x.shape
        M = A_mem0.shape[1]
        H, E = A_Wq.shape[1:]
        F = B_w1.shape[1]
        SEG = 32
        NP = H // 2
        NC = D // 128
        DM = NC * 128
        DP = DM + 128
        NW = (NC * H + NP) * 128
        LT = (M + SEG) // 8 * 128
        SC = cfg.get("sc", 128)
        any_spec = pl.BlockSpec(memory_space=pl.ANY)
        V = pltpu.VMEM
        outT = pl.pallas_call(
            make_kernel(S, D, H, E, M, SEG, F, cfg),
            in_specs=[any_spec] * 10,
            out_specs=any_spec,
            out_shape=jax.ShapeDtypeStruct((D, S), A_x.dtype),
            scratch_shapes=[
                V((D, S), BF16), V((M, D), BF16),
                V((NP, D, E), U32), V((NP, D, E), U32), V((NP, D, E), U32), V((H, D, E), BF16),
                V((S, F), BF16), V((F // 128, 128), BF16), V((F, S), BF16), V((S // 128, 128), BF16),
                V((9, H, 64, 128), U32), V((9, H, 64, 128), U32), V((6, 2 * H, 64, 128), U32),
                V((NP, DM // 2, 128), U32), V((NP, DM // 2, 128), U32), V((2, 2 * H, len(_HK_MIX), 64, 128), F32),
                V((NP, D // 2, 128), U32), V((NP, 64, DP), U32),
                V((NC + 1, S + 128, 128), F32), V((NC + 1, S + SEG, 128), F32),
                V((NC + 1, LT // 2, 128), U32), V((NC + 1, 64, LT), U32), V((NP, 64, 128), U32),
                V((NC + 1, LT // 2, 128), U32), V((4, NC + 1, SEG, 128), F32),
                V((2, NC + 1, 128, 128), F32), V((2, NC + 1, 128, 128), F32),
                V((DP, S), F32), V((DP, S), F32), V((D, F), F32), V((7, D // 4, F // 2), U32), V((D, S), BF16),
                pltpu.SemaphoreType.DMA((NP,)), pltpu.SemaphoreType.DMA((NP,)),
                pltpu.SemaphoreType.DMA((NP,)), pltpu.SemaphoreType.DMA((NP,)),
                pltpu.SemaphoreType.DMA((8,)), pltpu.SemaphoreType.DMA((S // SC,)),
            ],
            compiler_params=pltpu.CompilerParams(vmem_limit_bytes=110 * 1024 * 1024, flags=cfg.get("flags")),
        )(jnp.swapaxes(A_x[0], 0, 1), A_mem0[0], A_Wq, A_Wk, A_Wv, jnp.swapaxes(A_Wo, 1, 2),
          B_w1, B_b1.reshape(F // 128, 128), B_w2, B_b2.reshape(S // 128, 128))
        return jnp.swapaxes(outT, 0, 1)[None]
    return fn
STEPS = {"tail": 8, "recur": 56}


@jax.jit
def pallas_sequential_preLN__memory_aug_recurrent_mem_tr__mixer_token_mlp__prompt_kernel(
    A_x, A_mem0, A_Wq, A_Wk, A_Wv, A_Wo, A_seg_len, B_x, B_w1, B_b1, B_w2, B_b2,
):
    return build({})(A_x, A_mem0, A_Wq, A_Wk, A_Wv, A_Wo, A_seg_len, B_x, B_w1, B_b1, B_w2, B_b2)
```

```python
import contextlib
import functools
import math
import jax
import jax.numpy as jnp
from jax import lax
import jax.experimental.pallas as pl
import jax.experimental.pallas.tpu as pltpu

F32, BF16, U32 = jnp.float32, jnp.bfloat16, jnp.uint32
EPS = 1e-5

_dot = functools.partial(jnp.dot, preferred_element_type=F32)
_dot_nt = functools.partial(lax.dot_general, dimension_numbers=(((1,), (1,)), ((), ())),
                            preferred_element_type=F32)


def _split_pair(u):
    lo = pltpu.bitcast(u << 16, F32).astype(BF16)
    hi = pltpu.bitcast(u & jnp.uint32(0xFFFF0000), F32).astype(BF16)
    return lo, hi


def _pack(x):
    return x.astype(BF16)


def _pack2(a, b):
    return jnp.concatenate([a, b], axis=0).astype(BF16)


def _unpack(u):
    return pltpu.bitcast(u, BF16)


_HK_STEP = (
    (((1, 0, 0), (0, 0, 0)), ((1, 0, -1), (-1, 0, 0), (0, 0, 0)), ((1, 0, 0), (-1, 0, 0))),
    (((0, 1, 0), (0, 1, 0)), ((0, 0, 0), (-1, 1, 0), (0, -1, 0)), ((0, 1, 0), (0, 0, 0))),
    (((0, 0, 1), (0, 0, 0)), ((0, 0, 0), (0, 0, -1), (-1, 0, 1)), ((0, 0, 1), (0, 0, 0))),
    (((1, 1, 0), (0, 0, 0)), ((0, 0, 0), (1, 0, 0), (0, 0, 0)), ((1, 1, 0), (0, 0, 0))),
    (((1, 0, 0), (0, -1, 0)), ((0, 1, 0), (-1, 0, 0), (0, 0, 0)), ((0, 1, 0), (1, 0, 0))),
    (((1, 0, 1), (1, 0, 1)), ((0, 0, 0), (0, 0, 0), (1, 0, 0)), ((1, 0, 1), (0, 0, 0))),
    (((1, 0, 0), (1, 0, 1)), ((0, 0, 1), (0, 0, 0), (-1, 0, 0)), ((1, 0, 1), (-1, 0, 0))),
    (((0, 1, 1), (0, 0, 0)), ((0, 0, 0), (0, 0, 1), (0, 0, 0)), ((0, 1, 1), (0, -1, -1))),
    (((0, 1, 1), (0, 1, 0)), ((0, 0, 0), (0, 0, -1), (0, 1, 0)), ((0, 1, 0), (0, -1, -1))),
)
_HK_AHEAD = (
    (((1, 0, 0), (1, 0, 0)), ((1, -1, 0), (0, 0, 0), (-1, 0, 0)), ((0, 0, 0), (1, 0, 0))),
    (((0, 0, 0), (0, 1, 0)), ((0, 1, 0), (0, -1, 1), (0, 0, 0)), ((0, 1, 0), (0, -1, 0))),
    (((0, 0, 0), (0, 0, 1)), ((0, 0, -1), (0, 0, 0), (0, -1, 1)), ((0, 0, 0), (0, 0, 1))),
    (((0, 0, 0), (1, 1, 0)), ((0, 1, 0), (0, 0, 0), (0, 0, 0)), ((0, 0, 0), (1, 1, 0))),
    (((0, 0, 0), (1, 0, 1)), ((0, 0, -1), (0, 0, 0), (0, 0, 0)), ((1, 0, 1), (-1, 0, -1))),
    (((0, 1, 1), (0, 1, 1)), ((0, 0, 0), (0, 0, 0), (0, 1, 0)), ((0, 0, 0), (0, 1, 1))),
)
_HK_MIX = sorted({tuple(o[g][c] for _, _, o in _HK_AHEAD) for g in range(2) for c in range(3)}, reverse=True)
_HK_MIX_OF = [[_HK_MIX.index(tuple(o[g][c] for _, _, o in _HK_AHEAD)) for c in range(3)] for g in range(2)]


def _signed_sum(coefs, values):
    terms = sorted(((c, i) for i, c in enumerate(coefs) if c), key=lambda t: -t[0])
    acc = values[terms[0][1]] if terms[0][0] > 0 else -values[terms[0][1]]
    for c, i in terms[1:]:
        acc = acc + values[i] if c > 0 else acc - values[i]
    return acc


def _flat(rows):
    return [c for row in rows for c in row]


def _tiles(ref, lead, start, count, axis):
    words = ref.bitcast(U32)
    return _unpack(jnp.concatenate([words[(*lead, start + i)] for i in range(count)], axis=axis))


def _strassen_lhs(a11, a12, a21, a22):
    return [a11 + a22, a21 + a22, a11, a22, a11 + a12, a21 - a11, a12 - a22]


def _strassen_rhs(b11, b12, b21, b22):
    return [b11 + b22, b11, b12 - b22, b21 - b11, b22, b11 + b12, b21 + b22]


def _strassen_out(m1, m2, m3, m4, m5, m6, m7):
    return m1 + m4 - m5 + m7, m3 + m5, m2 + m4, m1 - m2 + m3 + m6


ORDER = ("H H H H km:02 G km:23 H km:35 !H km:58 t0 t1 t2 tl:03 !t0 tl:34 t3 q !t1 c !G a d s vm:07 f vm:78 "
         "N Z Z Z T X g !Z !N h !T !X b")
ORDER0 = ("H H H H km:02 G km:23 H km:35 !H km:58 t0 t1 t2 tl:03 !t0 tl:34 t3 q !t1 y !G d s vm:07 f vm:78 "
          "N T g !N h !T x")


def make_kernel(S, D, H, E, M, SEG, F, cfg):
    NP = H // 2
    NC = D // 128
    DM = NC * 128
    L = M + SEG
    G = L // 8
    TB = 128
    SPB = TB // SEG
    BLK = cfg.get("blk", 2)
    NB = S // TB
    NS = S // SEG
    scope = lambda name: jax.named_scope(name) if name in cfg.get("scopes", "") else contextlib.nullcontext()
    scale = (E ** -0.5) * math.log2(math.e)
    NCH = cfg.get("nch", 512)
    ZL = 16
    XL = ZL // SPB + 1
    LOOK = cfg.get("look", 2)

    def kernel(xT_h, mem_h, wq_h, wk_h, wv_h, woT_h, w1_h, b1_h, w2_h, b2_h, out_h,
               xT_s, mem_s, wq_s, wk_s, wv_s, wo_s, w1_s, b1_s, w2_s, b2_s,
               WS, WA, TQ, UNS, AH, WC, B2, X, Z, KT, KX, GX, VT, O, HS, NS_, hT, nT, U, GA, out_s,
               sem_q, sem_k, sem_v, sem_o, sem_m, sem_out):
        wq_u, wk_u, wv_u = (r.bitcast(U32) for r in (wq_h, wk_h, wv_h))
        def v_copies(p):
            return [pltpu.make_async_copy(wv_u.at[:, p, :], wv_s.at[p], sem_v.at[p]),
                    pltpu.make_async_copy(woT_h.at[pl.ds(2 * p, 2)], wo_s.at[pl.ds(2 * p, 2)], sem_o.at[p])]

        def k_copies(p):
            return [pltpu.make_async_copy(wq_u.at[:, p, :], wq_s.at[p], sem_q.at[p]),
                    pltpu.make_async_copy(wk_u.at[:, p, :], wk_s.at[p], sem_k.at[p])]

        def x_copy(b0, b1, sem):
            cols = pl.ds(b0 * TB, (b1 - b0) * TB)
            return pltpu.make_async_copy(xT_h.at[:, cols], xT_s.at[:, cols], sem)

        cp_x0 = x_copy(0, 2, sem_m.at[0])
        cp_x1 = x_copy(2, XL + 2, sem_m.at[1])
        cp_x2 = x_copy(XL + 2, NB, sem_m.at[7])
        cp_mem = pltpu.make_async_copy(mem_h, mem_s, sem_m.at[2])
        cp_w1 = pltpu.make_async_copy(w1_h, w1_s, sem_m.at[3])
        cp_w2 = pltpu.make_async_copy(w2_h, w2_s, sem_m.at[4])
        cp_b1 = pltpu.make_async_copy(b1_h, b1_s, sem_m.at[5])
        cp_b2 = pltpu.make_async_copy(b2_h, b2_s, sem_m.at[6])
        small = [cp_x0, cp_mem, cp_b1, cp_b2]
        for cp in small:
            cp.start()
        ALL = cfg.get("all", "kxv")
        for p in range(NP if "k" in ALL else LOOK):
            for cp in k_copies(p):
                cp.start()
        if "x" in ALL:
            cp_x1.start()
        for p in range(NP if "v" in ALL else 0):
            for cp in v_copies(p):
                cp.start()

        def start_pair(q):
            if "k" not in ALL:
                @pl.when(q < NP)
                def _():
                    for cp in k_copies(jnp.minimum(q, NP - 1)):
                        cp.start()

            if "x" not in ALL:
                @pl.when(q == NP)
                def _():
                    cp_x1.start()
                    if "w" in ALL:
                        for p in range(NP):
                            for cp in v_copies(p):
                                cp.start()

            if "v" not in ALL and "w" not in ALL:
                @pl.when(jnp.logical_and(q >= NP, q < 2 * NP))
                def _():
                    for cp in v_copies(jnp.clip(q - NP, 0, NP - 1)):
                        cp.start()

        lane = lax.broadcasted_iota(jnp.int32, (8, 128), 1)
        lo_half = lane < 64

        def lo_mask(n):
            return lax.broadcasted_iota(jnp.int32, (n, 128), 1) < 64

        def store_unit(cols, unit):
            blocks = [col[128 * k:128 * k + 128] for k in range(NC) for col in cols]
            for W, table in ((WS, _HK_STEP), (WA, _HK_AHEAD)):
                for r, (_, coefs, _) in enumerate(table):
                    W[r, unit] = _pack(_signed_sum(_flat(coefs), blocks))

        def store_head(y, unit):
            store_unit([y[:, 128 * c:128 * c + 128] for c in range(NC)], unit)

        def ahead(sb, hs, count, after=lambda v: v):
            base = pl.multiple_of(sb * 8 * SEG, 8 * SEG)
            x = [jnp.concatenate([Z[k, pl.ds(base + n * SEG + SEG - 16 + 8 * g, 8), :] for n in range(8)], axis=0)
                 for g in range(2) for k in range(NC)]
            w = [_tiles(WA, (r,), hs, count, 1) for r in range(len(_HK_AHEAD))]
            m = []
            for r, (coefs, _, _) in enumerate(_HK_AHEAD):
                yield
                m.append(_dot(after(_signed_sum(_flat(coefs), x)), w[r]))
            for n, coefs in enumerate(_HK_MIX):
                v = _signed_sum(coefs, m)
                for i in range(count):
                    AH[sb & 1, hs + i, n] = v[:, 128 * i:128 * i + 128]

        def x_piece(src, dst, j):
            r0 = pl.multiple_of(j * 128, 64)
            r1 = pl.multiple_of(jnp.minimum(j * 128 + 64, DM), 64)
            t = jnp.concatenate([xT_s[pl.ds(r0, 64), pl.ds(src, TB)], xT_s[pl.ds(r1, 64), pl.ds(src, TB)]], axis=0)
            X[j, pl.ds(dst, TB), :] = t.astype(F32).T

        def layernorm(tiles):
            mask = lo_mask(tiles[0].shape[0])

            def mean(ts):
                acc = functools.reduce(jnp.add, ts[:NC]) + jnp.where(mask, ts[NC], 0.0)
                return jnp.sum(acc, axis=1, keepdims=True) * (1.0 / D)

            m = mean(tiles)
            yield
            c = [t - m for t in tiles]
            v = mean([t * t for t in c])
            yield
            r = lax.rsqrt(v + EPS)
            return [t * r for t in c]

        def z_piece(src, dst, rows=SEG):
            z = yield from layernorm([X[c, pl.ds(src, rows), :] for c in range(NC + 1)])
            for c in range(NC + 1):
                Z[c, pl.ds(dst, rows), :] = z[c]

        def h_piece(t0, slot, dst_slot, dst):
            h = [X[c, pl.ds(t0, SEG), :] + O[slot, c] for c in range(NC + 1)]
            for c in range(NC + 1):
                HS[dst_slot, c, pl.ds(dst, SEG), :] = h[c]
            n = yield from layernorm(h)
            n = yield from layernorm(n)
            for c in range(NC + 1):
                NS_[dst_slot, c, pl.ds(dst, SEG), :] = n[c]

        def finish(gen):
            for _ in gen:
                pass

        def ht_piece(slot, col, j):
            hT[pl.ds(pl.multiple_of(j * 128, 128), 128), pl.ds(col, TB)] = HS[slot, j].T

        def nt_piece(slot, col, j):
            nT[pl.ds(pl.multiple_of(j * 128, 128), 128), pl.ds(col, TB)] = NS_[slot, j].T

        O[...] = jnp.zeros(O.shape, F32)
        HS[1] = jnp.zeros(HS.shape[1:], F32)
        NS_[...] = jnp.zeros(NS_.shape, F32)
        hT[0:TB, 0:128] = jnp.zeros((TB, 128), F32)
        nT[0:TB, 0:128] = jnp.zeros((TB, 128), F32)
        TQ[0, 2] = jnp.zeros((DM, 128), F32)

        def tail_first(w):
            return jnp.concatenate([w[DM:], w[:DM]], axis=0)

        def fold(l0, l1, r0, r1, late=lambda a: a):
            a0, a1 = tail_first(l0), tail_first(l1)

            def tail(n0, n1):
                return jnp.concatenate([_dot_nt(r0[DM:], l0[n0:n1]), _dot_nt(r1[DM:], l1[n0:n1])], axis=0)

            cut = cfg.get("cut", (256, D, D))
            y0a = _dot_nt(a0, r0[:256])
            ts = [tail(0, cut[0])]
            y0b, y1a = _dot_nt(a0, r0[256:DM]), _dot_nt(late(a1) if cfg.get("late") == 2 else a1, r1[:128])
            if cut[1] > cut[0]:
                ts.append(tail(cut[0], cut[1]))
            y1b = _dot_nt(late(a1), r1[128:DM])
            if cut[2] > cut[1]:
                ts.append(tail(cut[1], cut[2]))
            t = jnp.concatenate(ts + [jnp.zeros((128, 64), F32)], axis=1)
            return jnp.concatenate([y0a, y0b], axis=1), jnp.concatenate([y1a, y1b], axis=1), t

        def fold_k(p):
            y0, y1, t = fold(*_split_pair(wk_s[p]), *_split_pair(wq_s[p]))
            TQ[p, 0] = t[:, :DM].T
            corner = t[:64, DM:] + pltpu.roll(t[64:, DM:], 64, 1)
            WC[p] = _pack(corner)
            store_head(y0[64:], 2 * p)
            store_head(y1[64:], 2 * p + 1)
            TQ[p, 1] = jnp.concatenate([y0[:64], y1[:64]], axis=0).T

        def magnitude(x):
            m = functools.reduce(jnp.maximum, [jnp.abs(x[r:r + 8]) for r in range(0, x.shape[0], 8)])
            m = jnp.max(jnp.max(m, axis=0, keepdims=True), axis=1, keepdims=True)
            m = pltpu.bitcast(jnp.broadcast_to(m, (8, 128)), U32) & jnp.uint32(0x7F800000)
            return jnp.clip(pltpu.bitcast(m, F32), 2.0 ** -60, 2.0 ** 60)

        def store_narrow(p):
            tk, tq, tv = TQ[p, 0], TQ[p, 1], TQ[p, 2]
            mk, mv = magnitude(tk), magnitude(tv)
            UNS[p] = mv / mk
            store_unit([tk, tv * (mk / mv)[:1], tq], 2 * H + p)

        def fold_v(p, late):
            y0, y1, t = fold(*_split_pair(wv_s[p]), wo_s[2 * p], wo_s[2 * p + 1], late)
            t = t.T
            TQ[p, 2] = t[:DM]
            store_head(y0[64:], H + 2 * p)
            store_head(y1[64:], H + 2 * p + 1)
            m = lo_mask(64)
            top = jnp.concatenate([y0[:64], jnp.where(m, t[DM:D], 0.0)], axis=1)
            bot = jnp.concatenate([y1[:64], jnp.where(m, 0.0, t[DM:D])], axis=1)
            b2 = _pack(jnp.concatenate([top, bot], axis=0))
            for c in range(NC + 1):
                B2[c, p] = b2[:, 128 * c:128 * c + 128]

        def init_bias(n):
            b1 = b1_s[...].astype(F32)
            rows = lax.broadcasted_iota(jnp.int32, b1.shape, 0)
            per = pl.cdiv(F // 128, NP - 1)
            for k in range(per):
                r = jnp.minimum(n * per + k, F // 128 - 1)
                bias = jnp.sum(jnp.where(rows == r, b1, 0.0), axis=0, keepdims=True)
                U[:, pl.ds(pl.multiple_of(r * 128, 128), 128)] = jnp.broadcast_to(bias, (D, 128))

        def k_loop(p, _):
            for cp in k_copies(p):
                cp.wait()
            start_pair(p + LOOK)
            early = ahead(0, 2 * p - 2, 2)
            for _ in range(1 + cfg.get("pre", 0)):
                next(early)
            fold_k(p)
            init_bias(p - 1)
            finish(early)

        def v_loop(p, _):
            for cp in v_copies(p):
                cp.wait()
            if "w" not in ALL:
                start_pair(NP + p + LOOK)
            early = ahead(0, H + 2 * p - 2, 2)
            store_narrow(jnp.maximum(p - 1, 0))
            probe = WA[0, p, 0:16, :]
            next(early)

            def late(a):
                keep = lax.broadcasted_iota(jnp.int32, (16, 128), 1) < p + 128
                head = jnp.concatenate([jnp.where(keep, a[:16, :128], probe), a[:16, 128:]], axis=1)
                return jnp.concatenate([head, a[16:]], axis=0)

            fold_v(p, late if cfg.get("late", 1) else lambda a: a)
            finish(early)
            r = pl.multiple_of((8 + p) * SEG, SEG)
            finish(z_piece(r, r))
            c0 = pl.multiple_of((3 + (p >> 2)) * TB, TB)
            x_piece(c0, c0, p & 3)

        if cfg.get("only"):
            for cp in small + [cp_x1] + [c for p in range(NP) for c in k_copies(p) + v_copies(p)]:
                cp.wait()
        with scope("fold_k"):
          if not cfg.get("only"):
            for cp in small:
                cp.wait()
            for b in range(2):
                for j in range(NC + 1):
                    x_piece(b * TB, b * TB, j)
                finish(z_piece(b * TB, b * TB, TB))
            for cp in k_copies(0):
                cp.wait()
            if "k" not in ALL:
                for cp in k_copies(LOOK):
                    cp.start()
            fold_k(0)
            lax.fori_loop(1, NP, k_loop, None)
        with scope("fold_v"):
          if not cfg.get("only"):
            cp_x1.wait()
            for j in range(NC + 1):
                x_piece(2 * TB, 2 * TB, j)
            lax.fori_loop(0, NP, v_loop, None)
        if cfg.get("stop"):
            cp_x2 = cp_mem
            cp_w1 = cp_b1
            cp_w2 = cp_b2
        for cp in (cp_x2, cp_w1, cp_w2):
            cp.start()
        with scope("ahead0"):
            store_narrow(NP - 1)
            finish(ahead(0, 2 * H - 2, 2))
            for unit in range(2 * H, 2 * H + NP, 4):
                finish(ahead(0, unit, 4))
        if cfg.get("stop"):
            for cp in (cp_x2, cp_w1, cp_w2):
                cp.wait()
            return
        mem0 = mem_s[...].astype(F32)
        mem0 = jnp.concatenate([mem0, mem0[:, DM:]], axis=1)

        row = lax.broadcasted_iota(jnp.int32, (8, 128), 0)
        tri = row >= (lane & 7)
        blockid = lane >> 4

        def project(lhs, unit, early, after):
            m = [_dot(after(a), _tiles(WS, (r,), unit, 2, 1)) for r, a in enumerate(lhs)]
            last = [v[L - 16:] for v in m]
            out = []
            for c in range(NC):
                y = _signed_sum([o[0][c] for _, _, o in _HK_STEP], m)
                u = _signed_sum([o[1][c] for _, _, o in _HK_STEP], last)
                out.append([[y[8 * t:8 * t + 8, 128 * k:128 * k + 128] for t in range(G - 2)]
                            + [y[L - 16:, 128 * k:128 * k + 128] + early(unit + k, _HK_MIX_OF[0][c]),
                               u[:, 128 * k:128 * k + 128] + early(unit + k, _HK_MIX_OF[1][c])]
                            for k in range(2)])
            return out

        def project_main(lhs, T, side, early, after, lo, hi):
            for p in range(lo, hi):
                for c, (even, odd) in enumerate(project(lhs, side * H + 2 * p, early, after)):
                    for t in range(G):
                        T[c, t * 128 + 16 * p:t * 128 + 16 * p + 16, :] = _pack2(even[t], odd[t])

        def project_tail(lhs, st, early, after, lo, hi):
            for j in range(lo, hi):
                k3, v3, q = project(lhs, 2 * H + 2 * j, early, after)
                for k in range(2):
                    p = 2 * j + k
                    st["q1", p] = jnp.concatenate(q[k], axis=0)
                    for T, rows in ((KT, k3[k]), (VT, [v * UNS[p] for v in v3[k]])):
                        for t, v in enumerate(rows):
                            T[NC, t * 128 + 16 * p:t * 128 + 16 * p + 16, :] = _pack2(
                                jnp.where(lo_half, v, 0.0), jnp.where(lo_half, 0.0, v))

        def allreduce8(x, op):
            for k in (1, 2, 4):
                y = jnp.where((lane & k) != 0, pltpu.roll(x, k, 1), pltpu.roll(x, 128 - k, 1))
                x = op(x, y)
            return x

        def groups(t):
            if cfg.get("full"):
                return list(range(G))
            return [0] + list(range(max(min(t, cfg.get("tmax", 9)), 1), G))

        def ntiles(r):
            return G if r == 0 else r + 1

        def step(mem, s, side, probes, keep, order):
            t0 = pl.multiple_of(s * SEG, SEG)
            zt = [jnp.concatenate([mem[:, 128 * c:128 * c + 128], Z[c, pl.ds(t0, SEG), :]], axis=0) for c in range(NC + 1)]
            full = [v[:L - 8] for v in zt[:NC]]
            pair = [v[L - 16:L - 8] for v in zt[:NC]] + [v[L - 8:] for v in zt[:NC]]
            lhs = [jnp.concatenate([_signed_sum(coefs[0], [v[:L - 16] for v in full]), _signed_sum(_flat(coefs), pair)], axis=0)
                   for coefs, _, _ in _HK_STEP]
            lhs = [v.astype(BF16) for v in lhs]
            early = lambda hs, n: AH[(s >> 3) & 1, hs, n, pl.ds(pl.multiple_of((s & 7) * 8, 8), 8), :]
            zs = jnp.concatenate(zt, axis=1)
            z2 = zt[NC]
            g = [_pack2(jnp.where(lo_half, z2[8 * t:8 * t + 8], 0.0),
                        jnp.where(lo_half, 0.0, z2[8 * t:8 * t + 8])) for t in range(G)]
            zero = jnp.zeros((16, 128), BF16)
            Gp = [jnp.concatenate([g[(b - p) % NP] if (b - p) % NP < G else zero for b in range(NP)], axis=0)
                  for p in range(NP)]
            st = {"wait": []}

            def after(lhs):
                if not st["wait"]:
                    return lhs
                dt = lhs.dtype
                lhs = lhs.astype(F32)
                head = lhs[:8, :128]
                for v in st["wait"]:
                    head = jnp.where(keep, head, v)
                st["wait"] = []
                if lhs.shape[1] > 128:
                    head = jnp.concatenate([head, lhs[:8, 128:]], axis=1)
                return jnp.concatenate([head, lhs[8:]], axis=0).astype(dt)

            def q2_proj():
                st["q2"] = (jnp.concatenate([st["q1", p] for p in range(NP)], axis=1)
                            + _dot(after(zt[NC])[:, :64], _tiles(WC, (), 0, NP, 1)))

            mode = cfg.get("gx", "roll")

            def g_transpose():
                if mode == "nt":
                    return
                g0 = pltpu.bitcast(Gp[0].T, U32)
                for p in range(NP):
                    if mode == "roll":
                        GX[p] = pltpu.roll(g0, 16 * p, 1) if p else g0
                    else:
                        GX[p] = pltpu.bitcast(Gp[p].T, U32)

            def term2():
                q2 = st["q2"]
                if mode == "nt":
                    o = [_dot_nt(q2[:, 128 * p:128 * p + 128], Gp[p]) for p in range(NP)]
                else:
                    o = [_dot(after(q2[:, 128 * p:128 * p + 128]), _unpack(GX[p])) for p in range(NP)]
                extra = []
                for r in range(G):
                    rowt = []
                    for t in range(ntiles(r)):
                        x = o[0][8 * r:8 * r + 8]
                        for p in range(1, NP):
                            x = jnp.where(blockid == (p + t) % NP, o[p][8 * r:8 * r + 8], x)
                        rowt.append(pltpu.roll(x, 128 - 16 * t, 1) if t else x)
                    extra.append(rowt)
                st["extra"] = extra

            def k_transpose(c):
                KX[c] = pltpu.bitcast(_unpack(KT.bitcast(U32)[c]).T, U32)

            def scores():
                s = {}
                for t in range(G):
                    rs = groups(t)
                    lhs = after(jnp.concatenate([zs[8 * r:8 * r + 8] for r in rs], axis=0))
                    rhs = jnp.concatenate([_unpack(KX[c, :, 128 * t:128 * t + 128]) for c in range(NC + 1)], axis=0)
                    y = _dot(lhs, rhs)
                    for i, r in enumerate(rs):
                        s[r, t] = y[8 * i:8 * i + 8]
                pt = []
                for r in range(G):
                    tiles = [s[r, t] + st["extra"][r][t] for t in range(ntiles(r))]
                    if r > 0:
                        tiles[r] = jnp.where(tri, tiles[r], -1e9 * math.sqrt(E))
                    m = allreduce8(functools.reduce(jnp.maximum, tiles), jnp.maximum)
                    e = [jnp.exp2((x - m) * scale) for x in tiles]
                    l = allreduce8(functools.reduce(jnp.add, e), jnp.add)
                    inv = pl.reciprocal(l, approx=True)
                    inv = inv * (2.0 - l * inv)
                    for _ in range(cfg.get("pad", 0)):
                        inv = pltpu.roll(pltpu.roll(inv, 16, 1), 112, 1)
                    pt.append([x * inv for x in e])
                st["pt"] = pt

            def pz2():
                pt = st["pt"]
                sk = [[pltpu.roll(x, 16 * t, 1) if t else x for t, x in enumerate(rowt)] for rowt in pt]
                pz = []
                for p in range(NP):
                    rows = []
                    for r in range(G):
                        n = ntiles(r)
                        x = sk[r][0] if n == G else jnp.where(blockid == p, sk[r][0], 0.0)
                        for t in range(1, n):
                            x = jnp.where(blockid == (p + t) % NP, sk[r][t], x)
                        rows.append(x)
                    pz.append(_dot(after(jnp.concatenate(rows, axis=0)), Gp[p]))
                st["pz"] = jnp.concatenate(pz, axis=1)

            def b2():
                y = _dot(after(st["pz"]), jnp.concatenate([_tiles(B2, (c,), 0, NP, 0) for c in range(NC + 1)], axis=1))
                st["o"] = [y[8 * r:8 * r + 8] for r in range(G)]

            def pv():
                for t in range(G):
                    rs = groups(t)
                    zf = jnp.zeros((8, 128), F32)
                    lhs = after(jnp.concatenate([st["pt"][r][t] if t < ntiles(r) else zf for r in rs], axis=0))
                    rhs = jnp.concatenate([_unpack(VT.bitcast(U32)[c, 64 * t:64 * t + 64, :]) for c in range(NC + 1)], axis=1)
                    y = _dot(lhs, rhs)
                    for i, r in enumerate(rs):
                        st["o"][r] = st["o"][r] + y[8 * i:8 * i + 8]

            items = {"q": q2_proj, "G": g_transpose, "d": term2, "s": scores, "f": pz2, "g": b2, "h": pv,
                     "tl": functools.partial(project_tail, lhs, st, early, after),
                     "km": functools.partial(project_main, lhs, KT, 0, early, after),
                     "vm": functools.partial(project_main, lhs, VT, 1, early, after)}
            for c in range(NC + 1):
                items[f"t{c}"] = functools.partial(k_transpose, c)
            for name in order.split():
                if name[0] == "!":
                    if name[1] == "G":
                        st["wait"].append(pltpu.bitcast(GX[NP - 1, 56:64, :], F32))
                    elif name[1] == "t":
                        c = int(name[2])
                        st["wait"].append(pltpu.bitcast(KX[c, 56:64, 128 * (G - 1):], F32))
                    else:
                        st["wait"].append(probes[name[1:]]())
                elif ":" in name:
                    items[name[:2]](int(name[3]), int(name[4]))
                elif name in side:
                    side[name](after)
                else:
                    items[name]()
            o = jnp.concatenate(st["o"], axis=0)
            tail = o[:, DM:]
            o = jnp.concatenate([o[:, :DM], tail + pltpu.roll(tail, 64, 1)], axis=1)
            return o[:M], o[M:]

        DH, FH, SH = D // 2, F // 2, S // 2

        def segment(i, s, mem, extra, order):
            b, j = s >> 2, s & 3
            col = lambda blk: pl.multiple_of(jnp.clip(blk, 0, NB - 1) * TB, TB)
            sp = s - 1
            hp = h_piece(pl.multiple_of(jnp.maximum(sp, 0) * SEG, SEG), sp & 3, (sp >> 2) & 1,
                         pl.multiple_of((sp & 3) * SEG, SEG))
            zp = z_piece(pl.multiple_of(jnp.minimum(s + ZL, NS - 1) * SEG, SEG),
                         pl.multiple_of(jnp.minimum(s + ZL, NS) * SEG, SEG))
            side = {"H": lambda a: next(hp, None), "Z": lambda a: next(zp, None),
                    "T": lambda a: ht_piece(1 - (b & 1), col(b - 1), j),
                    "N": lambda a: nt_piece(1 - (b & 1), col(b - 1), j),
                    "X": lambda a: x_piece(col(b + XL), pl.multiple_of(jnp.minimum(b + XL, NB) * TB, TB), j), **extra}
            u = (i >> 1) & 1
            rows = lambda n: pl.ds(pl.multiple_of(((i >> 2) & (n // 8 - 1)) * 8, 8), 8)
            probes = {"H": lambda: NS_[u, 0, rows(TB), :], "Z": lambda: Z[i & 3, rows(TB), :],
                      "T": lambda: hT[rows(TB), 0:128], "N": lambda: nT[rows(TB), 0:128],
                      "X": lambda: X[i & 3, rows(TB), :]}
            mem, o = step(mem, s, side, probes, lane < i + 128, order)
            for c in range(NC + 1):
                O[s & 3, c] = o[:, 128 * c:128 * c + 128]
            return mem

        S1 = NS - 8
        UA = (2 * H + NP) // 8
        RC = D // SPB
        KL = (NS - S1) // SPB * TB

        def body(i, mem):
            @pl.when(i == 1)
            def _():
                cp_x2.wait()

            for jj in range(BLK):
                s = BLK * i + jj
                first = ((s >> 1) & 3) * 2 * UA
                work = lambda at, n, after: finish(ahead((s >> 3) + 1, first + at, n, after))
                extra = {"b": functools.partial(work, 4 * (jj & 1), 2), "c": functools.partial(work, 4 * (jj & 1) + 2, 2),
                         "a": lambda after: work(8, 2, after) if jj & 1 == cfg.get("aj", 0) else None}
                mem = segment(i, s, mem, extra, cfg.get("order", ORDER))
            return mem

        TBLK = cfg.get("tblk", 2)

        def tail_body(i, mem):
            for jj in range(TBLK):
                n = TBLK * i + jj

                def mix(c0, c1, after):
                    k0 = pl.multiple_of((n >> 2) * TB, TB)
                    r0 = pl.multiple_of((n & 3) * RC, 8)
                    U[pl.ds(r0, RC), c0:c1] += _dot(after(nT[pl.ds(r0, RC), pl.ds(k0, TB)]), w1_s[pl.ds(k0, TB), c0:c1])

                cut = cfg.get("xcut", 768)
                mem = segment(i, S1 + n, mem, {"y": functools.partial(mix, 0, cut), "x": functools.partial(mix, cut, F)}, cfg.get("order0", ORDER0))
            return mem

        with scope("recur"):
            mem = lax.fori_loop(0, cfg.get("only", S1 // BLK), body, mem0)
        if cfg.get("only"):
            cp_w1.wait()
            cp_w2.wait()
            return
        cp_w1.wait()
        with scope("tail"):
            lax.fori_loop(0, (NS - S1) // TBLK, tail_body, mem)
        cp_w2.wait()

        def rhs_quads(w, r0, rh, c0, ch, width):
            return _strassen_rhs(*[w[r0 + dr:r0 + dr + rh, c0 + dc:c0 + dc + width].astype(F32)
                                   for dr in (0, rh) for dc in (0, ch)])

        with scope("mix1"):
            last = (NB - 1) & 1
            KH = (S - KL) // 2
            finish(h_piece((NS - 1) * SEG, (NS - 1) & 3, last, (SPB - 1) * SEG))
            a11, a21 = nT[:DH, KL:KL + KH], nT[DH:D, KL:KL + KH]
            a3, a6 = a11.astype(BF16), (a21 - a11).astype(BF16)
            for t in range(0, FH, 128):
                w = rhs_quads(w1_s, KL, KH, t, FH, 128)
                m3 = _dot(a3, w[2].astype(BF16))
                U[:DH, FH + t:FH + t + 128] += m3
                U[DH:, FH + t:FH + t + 128] += m3 + _dot(a6, w[5].astype(BF16))
            for j in range(NC + 1):
                nt_piece(last, (NB - 1) * TB, j)
            for j in range(NC + 1):
                ht_piece(last, (NB - 1) * TB, j)
            a = [v.astype(BF16) for v in _strassen_lhs(a11, nT[:DH, KL + KH:], a21, nT[DH:D, KL + KH:])]
            for t in range(0, FH, 128):
                w = rhs_quads(w1_s, KL, KH, t, FH, 128)
                m1, m2, m4, m5, m7 = (_dot(a[k], w[k].astype(BF16)) for k in (0, 1, 3, 4, 6))
                u = (U[:DH, t:t + 128] + (m1 + m4 - m5 + m7), U[:DH, FH + t:FH + t + 128] + m5,
                     U[DH:, t:t + 128] + (m2 + m4), U[DH:, FH + t:FH + t + 128] + (m1 - m2))
                g = [jax.nn.gelu(v, approximate=True) for v in u]
                for k, v in enumerate(_strassen_lhs(*g)):
                    GA[k, :, t:t + 128] = v
        b2v = b2_s[...].astype(F32)
        SC = 128
        cps = []
        flush = cfg.get("flush", (3, 5, 7, 8))
        with scope("mix2"):
            for i, s0 in enumerate(range(0, SH, SC)):
                w = rhs_quads(w2_s, 0, FH, s0, SH, SC)
                m = [_dot(GA[k].astype(BF16), w[k].astype(BF16)) for k in range(7)]
                for q, y in enumerate(_strassen_out(*m)):
                    rs = slice((q >> 1) * DH, (q >> 1) * DH + DH)
                    c0 = (q & 1) * SH + s0
                    bias = jnp.concatenate([b2v[r:r + 1] for r in range(c0 // 128, (c0 + SC) // 128)], axis=1)
                    out_s[rs, c0:c0 + SC] = (y + bias + hT[rs, c0:c0 + SC]).astype(BF16)
                if i + 1 in flush:
                    first = max([0] + [n for n in flush if n <= i]) * SC
                    for half in range(2):
                        cols = pl.ds(half * SH + first, s0 + SC - first)
                        cp = pltpu.make_async_copy(out_s.at[:, cols], out_h.at[:, cols], sem_out.at[2 * i + half])
                        cp.start()
                        cps.append(cp)
        for cp in cps:
            cp.wait()

    return kernel


def build(cfg):
    def fn(A_x, A_mem0, A_Wq, A_Wk, A_Wv, A_Wo, A_seg_len, B_x, B_w1, B_b1, B_w2, B_b2):
        _, S, D = A_x.shape
        M = A_mem0.shape[1]
        H, E = A_Wq.shape[1:]
        F = B_w1.shape[1]
        SEG = 32
        NP = H // 2
        NC = D // 128
        DM = NC * 128
        DP = DM + 128
        NW = (NC * H + NP) * 128
        LT = (M + SEG) // 8 * 128
        SC = cfg.get("sc", 128)
        any_spec = pl.BlockSpec(memory_space=pl.ANY)
        V = pltpu.VMEM
        outT = pl.pallas_call(
            make_kernel(S, D, H, E, M, SEG, F, cfg),
            in_specs=[any_spec] * 10,
            out_specs=any_spec,
            out_shape=jax.ShapeDtypeStruct((D, S), A_x.dtype),
            scratch_shapes=[
                V((D, S), BF16), V((M, D), BF16),
                V((NP, D, E), U32), V((NP, D, E), U32), V((NP, D, E), U32), V((H, D, E), BF16),
                V((S, F), BF16), V((F // 128, 128), BF16), V((F, S), BF16), V((S // 128, 128), BF16),
                V((9, 2 * H + NP, 128, 128), BF16), V((6, 2 * H + NP, 128, 128), BF16),
                V((NP, 3, DM, 128), F32), V((NP, 8, 128), F32), V((2, 2 * H + NP, len(_HK_MIX), 64, 128), F32),
                V((NP, 64, 128), BF16), V((NC + 1, NP, 128, 128), BF16),
                V((NC + 1, S + 128, 128), F32), V((NC + 1, S + SEG, 128), F32),
                V((NC + 1, LT, 128), BF16), V((NC + 1, 64, LT), U32), V((NP, 64, 128), U32),
                V((NC + 1, LT, 128), BF16), V((4, NC + 1, SEG, 128), F32),
                V((2, NC + 1, 128, 128), F32), V((2, NC + 1, 128, 128), F32),
                V((DP, S), F32), V((DP, S), F32), V((D, F), F32), V((7, D // 2, F // 2), F32), V((D, S), BF16),
                pltpu.SemaphoreType.DMA((NP,)), pltpu.SemaphoreType.DMA((NP,)),
                pltpu.SemaphoreType.DMA((NP,)), pltpu.SemaphoreType.DMA((NP,)),
                pltpu.SemaphoreType.DMA((8,)), pltpu.SemaphoreType.DMA((S // SC,)),
            ],
            compiler_params=pltpu.CompilerParams(vmem_limit_bytes=110 * 1024 * 1024, flags=cfg.get("flags")),
        )(jnp.swapaxes(A_x[0], 0, 1), A_mem0[0], A_Wq, A_Wk, A_Wv, jnp.swapaxes(A_Wo, 1, 2),
          B_w1, B_b1.reshape(F // 128, 128), B_w2, B_b2.reshape(S // 128, 128))
        return jnp.swapaxes(outT, 0, 1)[None]
    return fn
STEPS = {"tail": 8, "recur": 56}


@jax.jit
def pallas_sequential_preLN__memory_aug_recurrent_mem_tr__mixer_token_mlp__prompt_kernel(
    A_x, A_mem0, A_Wq, A_Wk, A_Wv, A_Wo, A_seg_len, B_x, B_w1, B_b1, B_w2, B_b2,
):
    return build({})(A_x, A_mem0, A_Wq, A_Wk, A_Wv, A_Wo, A_seg_len, B_x, B_w1, B_b1, B_w2, B_b2)
```

```python
import functools
import math

import jax
import jax.numpy as jnp
from jax import lax
import jax.experimental.pallas as pl
import jax.experimental.pallas.tpu as pltpu

F32, BF16, U32 = jnp.float32, jnp.bfloat16, jnp.uint32
EPS = 1e-5
TILE = 128
CHUNK = 8

_dot = functools.partial(jnp.dot, preferred_element_type=F32)
_dot_nt = functools.partial(
    lax.dot_general, dimension_numbers=(((1,), (1,)), ((), ())), preferred_element_type=F32)

_HK_STEP = (
    (((1, 0, 0), (0, 0, 0)), ((1, 0, -1), (-1, 0, 0), (0, 0, 0)), ((1, 0, 0), (-1, 0, 0))),
    (((0, 1, 0), (0, 1, 0)), ((0, 0, 0), (-1, 1, 0), (0, -1, 0)), ((0, 1, 0), (0, 0, 0))),
    (((0, 0, 1), (0, 0, 0)), ((0, 0, 0), (0, 0, -1), (-1, 0, 1)), ((0, 0, 1), (0, 0, 0))),
    (((1, 1, 0), (0, 0, 0)), ((0, 0, 0), (1, 0, 0), (0, 0, 0)), ((1, 1, 0), (0, 0, 0))),
    (((1, 0, 0), (0, -1, 0)), ((0, 1, 0), (-1, 0, 0), (0, 0, 0)), ((0, 1, 0), (1, 0, 0))),
    (((1, 0, 1), (1, 0, 1)), ((0, 0, 0), (0, 0, 0), (1, 0, 0)), ((1, 0, 1), (0, 0, 0))),
    (((1, 0, 0), (1, 0, 1)), ((0, 0, 1), (0, 0, 0), (-1, 0, 0)), ((1, 0, 1), (-1, 0, 0))),
    (((0, 1, 1), (0, 0, 0)), ((0, 0, 0), (0, 0, 1), (0, 0, 0)), ((0, 1, 1), (0, -1, -1))),
    (((0, 1, 1), (0, 1, 0)), ((0, 0, 0), (0, 0, -1), (0, 1, 0)), ((0, 1, 0), (0, -1, -1))),
)
_HK_AHEAD = (
    (((1, 0, 0), (1, 0, 0)), ((1, -1, 0), (0, 0, 0), (-1, 0, 0)), ((0, 0, 0), (1, 0, 0))),
    (((0, 0, 0), (0, 1, 0)), ((0, 1, 0), (0, -1, 1), (0, 0, 0)), ((0, 1, 0), (0, -1, 0))),
    (((0, 0, 0), (0, 0, 1)), ((0, 0, -1), (0, 0, 0), (0, -1, 1)), ((0, 0, 0), (0, 0, 1))),
    (((0, 0, 0), (1, 1, 0)), ((0, 1, 0), (0, 0, 0), (0, 0, 0)), ((0, 0, 0), (1, 1, 0))),
    (((0, 0, 0), (1, 0, 1)), ((0, 0, -1), (0, 0, 0), (0, 0, 0)), ((1, 0, 1), (-1, 0, -1))),
    (((0, 1, 1), (0, 1, 1)), ((0, 0, 0), (0, 0, 0), (0, 1, 0)), ((0, 0, 0), (0, 1, 1))),
)
_HK_MIX = sorted({tuple(o[g][c] for _, _, o in _HK_AHEAD) for g in range(2) for c in range(3)}, reverse=True)
_HK_MIX_OF = [[_HK_MIX.index(tuple(o[g][c] for _, _, o in _HK_AHEAD)) for c in range(3)] for g in range(2)]


def _flat(rows):
    return [c for row in rows for c in row]


def _signed_sum(coefs, values):
    terms = sorted(((c, i) for i, c in enumerate(coefs) if c), key=lambda t: -t[0])
    acc = values[terms[0][1]] if terms[0][0] > 0 else -values[terms[0][1]]
    for c, i in terms[1:]:
        acc = acc + values[i] if c > 0 else acc - values[i]
    return acc


def _strassen_lhs(a11, a12, a21, a22):
    return [a11 + a22, a21 + a22, a11, a22, a11 + a12, a21 - a11, a12 - a22]


def _strassen_rhs(b11, b12, b21, b22):
    return [b11 + b22, b11, b12 - b22, b21 - b11, b22, b11 + b12, b21 + b22]


def _strassen_out(m1, m2, m3, m4, m5, m6, m7):
    return m1 + m4 - m5 + m7, m3 + m5, m2 + m4, m1 - m2 + m3 + m6


def _split_pair(words):
    lo = pltpu.bitcast(words << 16, F32).astype(BF16)
    hi = pltpu.bitcast(words & jnp.uint32(0xFFFF0000), F32).astype(BF16)
    return lo, hi


def _stack_bf16(a, b):
    return jnp.concatenate([a, b], axis=0).astype(BF16)


def _tiles(ref, lead, indices, axis):
    words = ref.bitcast(U32)
    return pltpu.bitcast(jnp.concatenate([words[(*lead, i)] for i in indices], axis=axis), BF16)


def _low_lanes(rows):
    return lax.broadcasted_iota(jnp.int32, (rows, TILE), 1) < TILE // 2


def _make_kernel(S, D, H, E, M, SEG, F):
    NP = H // 2
    NC = D // TILE
    DM = NC * TILE
    L = M + SEG
    G = L // 8
    SPB = TILE // SEG
    NB = S // TILE
    NS = S // SEG
    UNITS = 2 * H + NP
    ZL = 2 * CHUNK
    XL = ZL // SPB + 1
    S1 = NS - CHUNK
    KL = CHUNK // SPB * TILE
    RC = D // SPB
    DH, FH, SH = D // 2, F // 2, S // 2
    FLUSH = (3, 5, 7, 8)
    scale = E ** -0.5 * math.log2(math.e)

    def kernel(xT_h, mem_h, wq_h, wk_h, wv_h, woT_h, w1_h, b1_h, w2_h, b2_h, out_h,
               xT_s, mem_s, wq_s, wk_s, wv_s, wo_s, w1_s, b1_s, w2_s, b2_s,
               WS, WA, narrow, unscale, AH, WC, B2, X, Z, KT, KX, GX, VT, O, HS, NS_, hT, nT, U, GA, out_s,
               sem_q, sem_k, sem_v, sem_o, sem_m, sem_out):
        wq_u, wk_u, wv_u = (r.bitcast(U32) for r in (wq_h, wk_h, wv_h))

        def k_copies(p):
            return [pltpu.make_async_copy(wq_u.at[:, p, :], wq_s.at[p], sem_q.at[p]),
                    pltpu.make_async_copy(wk_u.at[:, p, :], wk_s.at[p], sem_k.at[p])]

        def v_copies(p):
            return [pltpu.make_async_copy(wv_u.at[:, p, :], wv_s.at[p], sem_v.at[p]),
                    pltpu.make_async_copy(woT_h.at[pl.ds(2 * p, 2)], wo_s.at[pl.ds(2 * p, 2)], sem_o.at[p])]

        def x_copy(b0, b1, sem):
            cols = pl.ds(b0 * TILE, (b1 - b0) * TILE)
            return pltpu.make_async_copy(xT_h.at[:, cols], xT_s.at[:, cols], sem)

        cp_x0 = x_copy(0, 3, sem_m.at[0])
        cp_x1 = x_copy(3, XL + 2, sem_m.at[1])
        cp_x2 = x_copy(XL + 2, NB, sem_m.at[2])
        cp_mem = pltpu.make_async_copy(mem_h, mem_s, sem_m.at[3])
        cp_b1 = pltpu.make_async_copy(b1_h, b1_s, sem_m.at[4])
        cp_b2 = pltpu.make_async_copy(b2_h, b2_s, sem_m.at[5])
        cp_w1 = pltpu.make_async_copy(w1_h, w1_s, sem_m.at[6])
        cp_w2 = pltpu.make_async_copy(w2_h, w2_s, sem_m.at[7])
        small = [cp_x0, cp_mem, cp_b1, cp_b2]
        for cp in small:
            cp.start()
        for p in range(NP):
            for cp in k_copies(p):
                cp.start()
        cp_x1.start()
        for p in range(NP):
            for cp in v_copies(p):
                cp.start()

        lane = lax.broadcasted_iota(jnp.int32, (8, TILE), 1)
        row = lax.broadcasted_iota(jnp.int32, (8, TILE), 0)
        low = lane < TILE // 2

        def transpose_x(src, dst, j):
            r0 = pl.multiple_of(j * TILE, 64)
            r1 = pl.multiple_of(jnp.minimum(j * TILE + 64, DM), 64)
            t = jnp.concatenate([xT_s[pl.ds(r0, 64), pl.ds(src, TILE)], xT_s[pl.ds(r1, 64), pl.ds(src, TILE)]], axis=0)
            X[j, pl.ds(dst, TILE), :] = t.astype(F32).T

        def layernorm(tiles):
            mask = _low_lanes(tiles[0].shape[0])

            def mean(ts):
                acc = functools.reduce(jnp.add, ts[:NC]) + jnp.where(mask, ts[NC], 0.0)
                return jnp.sum(acc, axis=1, keepdims=True) * (1.0 / D)

            m = mean(tiles)
            c = [t - m for t in tiles]
            r = lax.rsqrt(mean([t * t for t in c]) + EPS)
            return [t * r for t in c]

        def normalize_x(src, dst, rows):
            z = layernorm([X[c, pl.ds(src, rows), :] for c in range(NC + 1)])
            for c in range(NC + 1):
                Z[c, pl.ds(dst, rows), :] = z[c]

        def residual(t0, slot, dst_slot, dst):
            h = [X[c, pl.ds(t0, SEG), :] + O[slot, c] for c in range(NC + 1)]
            for c in range(NC + 1):
                HS[dst_slot, c, pl.ds(dst, SEG), :] = h[c]
            n = layernorm(layernorm(h))
            for c in range(NC + 1):
                NS_[dst_slot, c, pl.ds(dst, SEG), :] = n[c]

        def transpose_back(dst, src, slot, col, j):
            dst[pl.ds(pl.multiple_of(j * TILE, TILE), TILE), pl.ds(col, TILE)] = src[slot, j].T

        def ahead_weights(units):
            return [_tiles(WA, (r,), units, 1) for r in range(len(_HK_AHEAD))]

        def ahead(chunk, units, weights, after=lambda v: v):
            base = pl.multiple_of(chunk * CHUNK * SEG, CHUNK * SEG)
            x = [jnp.concatenate([Z[k, pl.ds(base + n * SEG + SEG - 16 + 8 * g, 8), :] for n in range(CHUNK)], axis=0)
                 for g in range(2) for k in range(NC)]
            m = [_dot(after(_signed_sum(_flat(coefs), x)), w) for w, (coefs, _, _) in zip(weights, _HK_AHEAD)]
            for n, coefs in enumerate(_HK_MIX):
                v = _signed_sum(coefs, m)
                for i, unit in enumerate(units):
                    AH[chunk & 1, unit, n] = v[:, TILE * i:TILE * (i + 1)]

        def store_unit(cols, unit):
            blocks = [col[TILE * k:TILE * (k + 1)] for k in range(NC) for col in cols]
            for W, table in ((WS, _HK_STEP), (WA, _HK_AHEAD)):
                for r, (_, coefs, _) in enumerate(table):
                    W[r, unit] = _signed_sum(_flat(coefs), blocks).astype(BF16)

        def store_head(y, unit):
            store_unit([y[:, TILE * c:TILE * (c + 1)] for c in range(NC)], unit)

        def fold(l0, l1, r0, r1, late=lambda a: a):
            a0, a1 = (jnp.concatenate([w[DM:], w[:DM]], axis=0) for w in (l0, l1))

            def rest(n0, n1):
                return jnp.concatenate([_dot_nt(r0[DM:], l0[n0:n1]), _dot_nt(r1[DM:], l1[n0:n1])], axis=0)

            y0a = _dot_nt(a0, r0[:2 * TILE])
            ta = rest(0, 2 * TILE)
            y0b, y1a = _dot_nt(a0, r0[2 * TILE:DM]), _dot_nt(a1, r1[:TILE])
            tb = rest(2 * TILE, D)
            y1b = _dot_nt(late(a1), r1[TILE:DM])
            t = jnp.concatenate([ta, tb, jnp.zeros((TILE, 64), F32)], axis=1)
            return jnp.concatenate([y0a, y0b], axis=1), jnp.concatenate([y1a, y1b], axis=1), t

        def magnitude(x):
            m = functools.reduce(jnp.maximum, [jnp.abs(x[r:r + 8]) for r in range(0, x.shape[0], 8)])
            m = jnp.max(jnp.max(m, axis=0, keepdims=True), axis=1, keepdims=True)
            m = pltpu.bitcast(jnp.broadcast_to(m, (8, TILE)), U32) & jnp.uint32(0x7F800000)
            return jnp.clip(pltpu.bitcast(m, F32), 2.0 ** -60, 2.0 ** 60)

        def store_narrow(p):
            tk, tq, tv = narrow[p, 0], narrow[p, 1], narrow[p, 2]
            mk, mv = magnitude(tk), magnitude(tv)
            unscale[p] = mv / mk
            store_unit([tk, tv * (mk / mv)[:1], tq], 2 * H + p)

        def fold_keys(p, _):
            for cp in k_copies(p):
                cp.wait()
            before = jnp.maximum(p - 1, 0)
            units = (2 * before, 2 * before + 1)
            weights = ahead_weights(units)
            y0, y1, t = fold(*_split_pair(wk_s[p]), *_split_pair(wq_s[p]))
            narrow[p, 0] = t[:, :DM].T
            WC[p] = (t[:64, DM:] + pltpu.roll(t[64:, DM:], 64, 1)).astype(BF16)
            store_head(y0[64:], 2 * p)
            store_head(y1[64:], 2 * p + 1)
            narrow[p, 1] = jnp.concatenate([y0[:64], y1[:64]], axis=0).T
            b1 = b1_s[...].astype(F32)
            rows = lax.broadcasted_iota(jnp.int32, b1.shape, 0)
            per = pl.cdiv(F // TILE, NP)
            for k in range(per):
                r = jnp.minimum(p * per + k, F // TILE - 1)
                bias = jnp.sum(jnp.where(rows == r, b1, 0.0), axis=0, keepdims=True)
                U[:, pl.ds(pl.multiple_of(r * TILE, TILE), TILE)] = jnp.broadcast_to(bias, (D, TILE))
            ahead(0, units, weights)

        def fold_values(p, _):
            for cp in v_copies(p):
                cp.wait()
            store_narrow(jnp.maximum(p - 1, 0))
            probe = WA[0, p, 0:16, :]
            units = (H + 2 * p - 2, H + 2 * p - 1)
            weights = ahead_weights(units)

            def late(a):
                keep = lax.broadcasted_iota(jnp.int32, (16, TILE), 1) < p + TILE
                head = jnp.concatenate([jnp.where(keep, a[:16, :TILE], probe), a[:16, TILE:]], axis=1)
                return jnp.concatenate([head, a[16:]], axis=0)

            y0, y1, t = fold(*_split_pair(wv_s[p]), wo_s[2 * p], wo_s[2 * p + 1], late)
            t = t.T
            narrow[p, 2] = t[:DM]
            store_head(y0[64:], H + 2 * p)
            store_head(y1[64:], H + 2 * p + 1)
            m = _low_lanes(64)
            top = jnp.concatenate([y0[:64], jnp.where(m, t[DM:D], 0.0)], axis=1)
            bot = jnp.concatenate([y1[:64], jnp.where(m, 0.0, t[DM:D])], axis=1)
            b2 = _stack_bf16(top, bot)
            for c in range(NC + 1):
                B2[c, p] = b2[:, TILE * c:TILE * (c + 1)]
            ahead(0, units, weights)
            r = pl.multiple_of((CHUNK + p) * SEG, SEG)
            normalize_x(r, r, SEG)
            c0 = pl.multiple_of((3 + (p >> 2)) * TILE, TILE)
            transpose_x(c0, c0, p & 3)

        O[...] = jnp.zeros(O.shape, F32)
        HS[1] = jnp.zeros(HS.shape[1:], F32)
        NS_[...] = jnp.zeros(NS_.shape, F32)
        hT[0:TILE, 0:TILE] = jnp.zeros((TILE, TILE), F32)
        nT[0:TILE, 0:TILE] = jnp.zeros((TILE, TILE), F32)
        narrow[0, 2] = jnp.zeros((DM, TILE), F32)
        WA[:, 0:2] = jnp.zeros((len(_HK_AHEAD), 2, TILE, TILE), BF16)

        for cp in small:
            cp.wait()
        for b in range(3):
            for j in range(NC + 1):
                transpose_x(b * TILE, b * TILE, j)
            if b < 2:
                normalize_x(b * TILE, b * TILE, TILE)
        lax.fori_loop(0, NP, fold_keys, None)
        cp_x1.wait()
        lax.fori_loop(0, NP, fold_values, None)
        for cp in (cp_x2, cp_w1, cp_w2):
            cp.start()
        store_narrow(NP - 1)
        for units in ((2 * H - 2, 2 * H - 1), range(2 * H, 2 * H + NP // 2), range(2 * H + NP // 2, UNITS)):
            ahead(0, units, ahead_weights(units))

        causal = row >= (lane & 7)
        pair_of_lane = lane >> 4

        def over_keys(x, op):
            for k in (1, 2, 4):
                x = op(x, jnp.where((lane & k) != 0, pltpu.roll(x, k, 1), pltpu.roll(x, TILE - k, 1)))
            return x

        def queries_of(t):
            return [0] + list(range(max(t, 1), G))

        def keys_of(r):
            return G if r == 0 else r + 1

        def segment(i, s, mem, fill_mid, fill_end, run_ahead):
            t0 = pl.multiple_of(s * SEG, SEG)
            zt = [jnp.concatenate([mem[:, TILE * c:TILE * (c + 1)], Z[c, pl.ds(t0, SEG), :]], axis=0)
                  for c in range(NC + 1)]
            zs = jnp.concatenate(zt, axis=1)
            shared = [v[L - 16:L - 8] for v in zt[:NC]] + [v[L - 8:] for v in zt[:NC]]
            lhs = [jnp.concatenate([_signed_sum(coefs[0], [v[:L - 16] for v in zt[:NC]]),
                                    _signed_sum(_flat(coefs), shared)], axis=0).astype(BF16)
                   for coefs, _, _ in _HK_STEP]
            early = lambda unit, n: AH[(s >> 3) & 1, unit, n, pl.ds(pl.multiple_of((s & 7) * 8, 8), 8), :]
            g = [_stack_bf16(jnp.where(low, zt[NC][8 * t:8 * t + 8], 0.0), jnp.where(low, 0.0, zt[NC][8 * t:8 * t + 8]))
                 for t in range(G)]
            zero = jnp.zeros((16, TILE), BF16)
            tails = [jnp.concatenate([g[(b - p) % NP] if (b - p) % NP < G else zero for b in range(NP)], axis=0)
                     for p in range(NP)]

            keep = lane < i + TILE
            pinned = []
            slot = (i >> 1) & 1
            some_rows = pl.ds(pl.multiple_of(((i >> 2) & (TILE // 8 - 1)) * 8, 8), 8)

            def after(a):
                if not pinned:
                    return a
                wide = a.astype(F32)
                head = wide[:8, :TILE]
                for v in pinned:
                    head = jnp.where(keep, head, v)
                pinned.clear()
                if a.shape[1] > TILE:
                    head = jnp.concatenate([head, wide[:8, TILE:]], axis=1)
                return jnp.concatenate([head, wide[8:]], axis=0).astype(a.dtype)

            def project(unit):
                m = [_dot(after(a), _tiles(WS, (r,), (unit, unit + 1), 1)) for r, a in enumerate(lhs)]
                last = [v[L - 16:] for v in m]
                out = []
                for c in range(NC):
                    y = _signed_sum([o[0][c] for _, _, o in _HK_STEP], m)
                    u = _signed_sum([o[1][c] for _, _, o in _HK_STEP], last)
                    out.append([[y[8 * t:8 * t + 8, TILE * k:TILE * (k + 1)] for t in range(G - 2)]
                                + [y[L - 16:, TILE * k:TILE * (k + 1)] + early(unit + k, _HK_MIX_OF[0][c]),
                                   u[:, TILE * k:TILE * (k + 1)] + early(unit + k, _HK_MIX_OF[1][c])]
                                for k in range(2)])
                return out

            def project_heads(T, first, p0, p1):
                for p in range(p0, p1):
                    for c, (even, odd) in enumerate(project(first + 2 * p)):
                        for t in range(G):
                            T[c, t * TILE + 16 * p:t * TILE + 16 * (p + 1), :] = _stack_bf16(even[t], odd[t])

            q_tail = [None] * NP

            def project_narrow(j0, j1):
                for j in range(j0, j1):
                    k3, v3, q = project(2 * H + 2 * j)
                    for k in range(2):
                        p = 2 * j + k
                        q_tail[p] = jnp.concatenate(q[k], axis=0)
                        for T, rows in ((KT, k3[k]), (VT, [v * unscale[p] for v in v3[k]])):
                            for t, v in enumerate(rows):
                                T[NC, t * TILE + 16 * p:t * TILE + 16 * (p + 1), :] = _stack_bf16(
                                    jnp.where(low, v, 0.0), jnp.where(low, 0.0, v))

            def transpose_keys(c):
                KX[c] = pltpu.bitcast(pltpu.bitcast(KT.bitcast(U32)[c], BF16).T, U32)

            b, j = s >> 2, s & 3
            col = lambda blk: pl.multiple_of(jnp.clip(blk, 0, NB - 1) * TILE, TILE)
            sp = s - 1
            residual(pl.multiple_of(jnp.maximum(sp, 0) * SEG, SEG), sp & 3, (sp >> 2) & 1,
                     pl.multiple_of((sp & 3) * SEG, SEG))

            project_heads(KT, 0, 0, 2)
            g0 = pltpu.bitcast(tails[0].T, U32)
            for p in range(NP):
                GX[p] = pltpu.roll(g0, 16 * p, 1) if p else g0
            project_heads(KT, 0, 2, 5)
            pinned.append(NS_[slot, 0, some_rows, :])
            project_heads(KT, 0, 5, NP)
            for c in range(NC):
                transpose_keys(c)
            project_narrow(0, 3)
            pinned.append(pltpu.bitcast(KX[0, 56:64, TILE * (G - 1):], F32))
            project_narrow(3, NP // 2)
            transpose_keys(NC)
            q2 = jnp.concatenate(q_tail, axis=1) + _dot(after(zt[NC])[:, :64], _tiles(WC, (), range(NP), 1))
            pinned.append(pltpu.bitcast(KX[1, 56:64, TILE * (G - 1):], F32))
            fill_mid(after, lambda: pinned.append(pltpu.bitcast(GX[NP - 1, 56:64, :], F32)))

            o = [_dot(after(q2[:, TILE * p:TILE * (p + 1)]), pltpu.bitcast(GX[p], BF16)) for p in range(NP)]
            extra = []
            for r in range(G):
                extra.append([])
                for t in range(keys_of(r)):
                    x = o[0][8 * r:8 * r + 8]
                    for p in range(1, NP):
                        x = jnp.where(pair_of_lane == (p + t) % NP, o[p][8 * r:8 * r + 8], x)
                    extra[r].append(pltpu.roll(x, TILE - 16 * t, 1) if t else x)
            scores = {}
            for t in range(G):
                rs = queries_of(t)
                a = after(jnp.concatenate([zs[8 * r:8 * r + 8] for r in rs], axis=0))
                y = _dot(a, jnp.concatenate([pltpu.bitcast(KX[c, :, TILE * t:TILE * (t + 1)], BF16)
                                             for c in range(NC + 1)], axis=0))
                for n, r in enumerate(rs):
                    scores[r, t] = y[8 * n:8 * n + 8]
            probs = []
            for r in range(G):
                tiles = [scores[r, t] + extra[r][t] for t in range(keys_of(r))]
                if r > 0:
                    tiles[r] = jnp.where(causal, tiles[r], -1e9 * math.sqrt(E))
                m = over_keys(functools.reduce(jnp.maximum, tiles), jnp.maximum)
                e = [jnp.exp2((x - m) * scale) for x in tiles]
                total = over_keys(functools.reduce(jnp.add, e), jnp.add)
                inv = pl.reciprocal(total, approx=True)
                inv = inv * (2.0 - total * inv)
                probs.append([x * inv for x in e])

            project_heads(VT, H, 0, NP - 1)
            rotated = [[pltpu.roll(x, 16 * t, 1) if t else x for t, x in enumerate(tiles)] for tiles in probs]
            pz = []
            for p in range(NP):
                rows = []
                for r in range(G):
                    n = keys_of(r)
                    x = rotated[r][0] if n == G else jnp.where(pair_of_lane == p, rotated[r][0], 0.0)
                    for t in range(1, n):
                        x = jnp.where(pair_of_lane == (p + t) % NP, rotated[r][t], x)
                    rows.append(x)
                pz.append(_dot(after(jnp.concatenate(rows, axis=0)), tails[p]))
            project_heads(VT, H, NP - 1, NP)
            transpose_back(nT, NS_, 1 - (b & 1), col(b - 1), j)
            if run_ahead:
                normalize_x(pl.multiple_of(jnp.minimum(s + ZL, NS - 1) * SEG, SEG),
                            pl.multiple_of(jnp.minimum(s + ZL, NS) * SEG, SEG), SEG)
            transpose_back(hT, HS, 1 - (b & 1), col(b - 1), j)
            if run_ahead:
                transpose_x(col(b + XL), pl.multiple_of(jnp.minimum(b + XL, NB) * TILE, TILE), j)
            y = _dot(after(jnp.concatenate(pz, axis=1)),
                     jnp.concatenate([_tiles(B2, (c,), range(NP), 0) for c in range(NC + 1)], axis=1))
            out = [y[8 * r:8 * r + 8] for r in range(G)]
            if run_ahead:
                pinned.extend([Z[i & 3, some_rows, :], nT[some_rows, 0:TILE]])
            else:
                pinned.extend([nT[some_rows, 0:TILE], hT[some_rows, 0:TILE]])
            for t in range(G):
                rs = queries_of(t)
                a = after(jnp.concatenate([probs[r][t] for r in rs], axis=0))
                y = _dot(a, jnp.concatenate([pltpu.bitcast(VT.bitcast(U32)[c, 64 * t:64 * t + 64, :], BF16)
                                             for c in range(NC + 1)], axis=1))
                for n, r in enumerate(rs):
                    out[r] = out[r] + y[8 * n:8 * n + 8]
            if run_ahead:
                pinned.extend([hT[some_rows, 0:TILE], X[i & 3, some_rows, :]])
            fill_end(after)

            out = jnp.concatenate(out, axis=0)
            tail = out[:, DM:]
            out = jnp.concatenate([out[:, :DM], tail + pltpu.roll(tail, 64, 1)], axis=1)
            for c in range(NC + 1):
                O[s & 3, c] = out[M:, TILE * c:TILE * (c + 1)]
            return out[:M]

        def two_segments(i, mem):
            first = (i & 3) * (UNITS // 4)
            for n in range(2):
                s = 2 * i + n

                def work(at, after):
                    units = (first + at, first + at + 1)
                    ahead((s >> 3) + 1, units, ahead_weights(units), after)

                def fill_mid(after, pin):
                    work(4 * n + 2, after)
                    pin()
                    if n == 0:
                        work(8, after)

                mem = segment(i, s, mem, fill_mid, functools.partial(work, 4 * n), True)
            return mem

        def two_last_segments(i, mem):
            for n in range(2):
                k0 = pl.multiple_of(((2 * i + n) >> 2) * TILE, TILE)
                r0 = pl.multiple_of(((2 * i + n) & 3) * RC, 8)

                def mix(c0, c1, after):
                    U[pl.ds(r0, RC), c0:c1] += _dot(after(nT[pl.ds(r0, RC), pl.ds(k0, TILE)]), w1_s[pl.ds(k0, TILE), c0:c1])

                def fill_mid(after, pin):
                    mix(0, 6 * TILE, after)
                    pin()

                mem = segment(i, S1 + 2 * i + n, mem, fill_mid, functools.partial(mix, 6 * TILE, F), False)
            return mem

        def two_segments_after_copy(i, mem):
            pl.when(i == 1)(cp_x2.wait)
            return two_segments(i, mem)

        mem = mem_s[...].astype(F32)
        mem = jnp.concatenate([mem, mem[:, DM:]], axis=1)
        mem = lax.fori_loop(0, S1 // 2, two_segments_after_copy, mem)
        cp_w1.wait()
        lax.fori_loop(0, CHUNK // 2, two_last_segments, mem)
        cp_w2.wait()

        def strassen_operands(w, r0, rh, c0, ch):
            return _strassen_rhs(*[w[r0 + dr:r0 + dr + rh, c0 + dc:c0 + dc + TILE].astype(F32)
                                   for dr in (0, rh) for dc in (0, ch)])

        last = (NB - 1) & 1
        KH = (S - KL) // 2
        residual((NS - 1) * SEG, (NS - 1) & 3, last, (SPB - 1) * SEG)
        a11, a21 = nT[:DH, KL:KL + KH], nT[DH:D, KL:KL + KH]
        a3, a6 = a11.astype(BF16), (a21 - a11).astype(BF16)
        for t in range(0, FH, TILE):
            w = strassen_operands(w1_s, KL, KH, t, FH)
            m3 = _dot(a3, w[2].astype(BF16))
            U[:DH, FH + t:FH + t + TILE] += m3
            U[DH:, FH + t:FH + t + TILE] += m3 + _dot(a6, w[5].astype(BF16))
        for dst, src in ((nT, NS_), (hT, HS)):
            for j in range(NC + 1):
                transpose_back(dst, src, last, (NB - 1) * TILE, j)
        a = [v.astype(BF16) for v in _strassen_lhs(a11, nT[:DH, KL + KH:], a21, nT[DH:D, KL + KH:])]
        for t in range(0, FH, TILE):
            w = strassen_operands(w1_s, KL, KH, t, FH)
            m1, m2, m4, m5, m7 = (_dot(a[k], w[k].astype(BF16)) for k in (0, 1, 3, 4, 6))
            u = (U[:DH, t:t + TILE] + (m1 + m4 - m5 + m7), U[:DH, FH + t:FH + t + TILE] + m5,
                 U[DH:, t:t + TILE] + (m2 + m4), U[DH:, FH + t:FH + t + TILE] + (m1 - m2))
            for k, v in enumerate(_strassen_lhs(*[jax.nn.gelu(v, approximate=True) for v in u])):
                GA[k, :, t:t + TILE] = v

        b2 = b2_s[...].astype(F32)
        copies = []
        for f, (n0, n1) in enumerate(zip((0,) + FLUSH[:-1], FLUSH)):
            for n in range(n0, n1):
                w = strassen_operands(w2_s, 0, FH, n * TILE, SH)
                m = [_dot(GA[k].astype(BF16), w[k].astype(BF16)) for k in range(7)]
                for q, y in enumerate(_strassen_out(*m)):
                    rs = slice((q >> 1) * DH, (q >> 1) * DH + DH)
                    tile = (q & 1) * (SH // TILE) + n
                    cs = slice(tile * TILE, (tile + 1) * TILE)
                    out_s[rs, cs] = (y + b2[tile:tile + 1] + hT[rs, cs]).astype(BF16)
            for half in range(2):
                cols = pl.ds(half * SH + n0 * TILE, (n1 - n0) * TILE)
                copies.append(pltpu.make_async_copy(out_s.at[:, cols], out_h.at[:, cols], sem_out.at[2 * f + half]))
                copies[-1].start()
        for cp in copies:
            cp.wait()

    return kernel


@functools.partial(jax.jit, static_argnames=("A_seg_len",))
def pallas_sequential_preLN__memory_aug_recurrent_mem_tr__mixer_token_mlp__prompt_kernel(
    A_x, A_mem0, A_Wq, A_Wk, A_Wv, A_Wo, A_seg_len, B_x, B_w1, B_b1, B_w2, B_b2,
):
    del B_x
    B, S, D = A_x.shape
    M = A_mem0.shape[1]
    H, E = A_Wq.shape[1:]
    F = B_w1.shape[1]
    SEG = int(A_seg_len)
    assert (B, S, D, M, H, E, F, SEG) == (1, 2048, 448, 8, 16, 256, 1792, 32), "the tiling is laid out for these sizes"
    NP = H // 2
    NC = D // TILE
    DM = NC * TILE
    LT = (M + SEG) // 8 * TILE
    UNITS = 2 * H + NP
    vmem = pltpu.VMEM
    dma = pltpu.SemaphoreType.DMA
    in_hbm = pl.BlockSpec(memory_space=pl.ANY)
    outT = pl.pallas_call(
        _make_kernel(S, D, H, E, M, SEG, F),
        in_specs=[in_hbm] * 10,
        out_specs=in_hbm,
        out_shape=jax.ShapeDtypeStruct((D, S), A_x.dtype),
        scratch_shapes=[
            vmem((D, S), BF16),
            vmem((M, D), BF16),
            vmem((NP, D, E), U32), vmem((NP, D, E), U32), vmem((NP, D, E), U32),
            vmem((H, D, E), BF16),
            vmem((S, F), BF16), vmem((F // TILE, TILE), BF16),
            vmem((F, S), BF16), vmem((S // TILE, TILE), BF16),
            vmem((len(_HK_STEP), UNITS, TILE, TILE), BF16),
            vmem((len(_HK_AHEAD), UNITS, TILE, TILE), BF16),
            vmem((NP, 3, DM, TILE), F32),
            vmem((NP, 8, TILE), F32),
            vmem((2, UNITS, len(_HK_MIX), CHUNK * 8, TILE), F32),
            vmem((NP, 64, TILE), BF16),
            vmem((NC + 1, NP, TILE, TILE), BF16),
            vmem((NC + 1, S + TILE, TILE), F32),
            vmem((NC + 1, S + SEG, TILE), F32),
            vmem((NC + 1, LT, TILE), BF16),
            vmem((NC + 1, 64, LT), U32),
            vmem((NP, 64, TILE), U32),
            vmem((NC + 1, LT, TILE), BF16),
            vmem((4, NC + 1, SEG, TILE), F32),
            vmem((2, NC + 1, TILE, TILE), F32),
            vmem((2, NC + 1, TILE, TILE), F32),
            vmem((DM + TILE, S), F32),
            vmem((DM + TILE, S), F32),
            vmem((D, F), F32),
            vmem((7, D // 2, F // 2), F32),
            vmem((D, S), BF16),
            dma((NP,)), dma((NP,)), dma((NP,)), dma((NP,)), dma((8,)), dma((8,)),
        ],
        compiler_params=pltpu.CompilerParams(vmem_limit_bytes=110 * 1024 * 1024),
    )(jnp.swapaxes(A_x[0], 0, 1), A_mem0[0], A_Wq, A_Wk, A_Wv, jnp.swapaxes(A_Wo, 1, 2),
      B_w1, B_b1.reshape(F // TILE, TILE), B_w2, B_b2.reshape(S // TILE, TILE))
    return jnp.swapaxes(outT, 0, 1)[None]
```

```python
import functools
import math

import jax
import jax.numpy as jnp
from jax import lax
import jax.experimental.pallas as pl
import jax.experimental.pallas.tpu as pltpu

F32, BF16, U32 = jnp.float32, jnp.bfloat16, jnp.uint32
EPS = 1e-5
TILE = 128
CHUNK = 8

_dot = functools.partial(jnp.dot, preferred_element_type=F32)
_dot_nt = functools.partial(
    lax.dot_general, dimension_numbers=(((1,), (1,)), ((), ())), preferred_element_type=F32)

_HK_STEP = (
    (((1, 0, 0), (0, 0, 0)), ((1, 0, -1), (-1, 0, 0), (0, 0, 0)), ((1, 0, 0), (-1, 0, 0))),
    (((0, 1, 0), (0, 1, 0)), ((0, 0, 0), (-1, 1, 0), (0, -1, 0)), ((0, 1, 0), (0, 0, 0))),
    (((0, 0, 1), (0, 0, 0)), ((0, 0, 0), (0, 0, -1), (-1, 0, 1)), ((0, 0, 1), (0, 0, 0))),
    (((1, 1, 0), (0, 0, 0)), ((0, 0, 0), (1, 0, 0), (0, 0, 0)), ((1, 1, 0), (0, 0, 0))),
    (((1, 0, 0), (0, -1, 0)), ((0, 1, 0), (-1, 0, 0), (0, 0, 0)), ((0, 1, 0), (1, 0, 0))),
    (((1, 0, 1), (1, 0, 1)), ((0, 0, 0), (0, 0, 0), (1, 0, 0)), ((1, 0, 1), (0, 0, 0))),
    (((1, 0, 0), (1, 0, 1)), ((0, 0, 1), (0, 0, 0), (-1, 0, 0)), ((1, 0, 1), (-1, 0, 0))),
    (((0, 1, 1), (0, 0, 0)), ((0, 0, 0), (0, 0, 1), (0, 0, 0)), ((0, 1, 1), (0, -1, -1))),
    (((0, 1, 1), (0, 1, 0)), ((0, 0, 0), (0, 0, -1), (0, 1, 0)), ((0, 1, 0), (0, -1, -1))),
)
_HK_AHEAD = (
    (((1, 0, 0), (1, 0, 0)), ((1, -1, 0), (0, 0, 0), (-1, 0, 0)), ((0, 0, 0), (1, 0, 0))),
    (((0, 0, 0), (0, 1, 0)), ((0, 1, 0), (0, -1, 1), (0, 0, 0)), ((0, 1, 0), (0, -1, 0))),
    (((0, 0, 0), (0, 0, 1)), ((0, 0, -1), (0, 0, 0), (0, -1, 1)), ((0, 0, 0), (0, 0, 1))),
    (((0, 0, 0), (1, 1, 0)), ((0, 1, 0), (0, 0, 0), (0, 0, 0)), ((0, 0, 0), (1, 1, 0))),
    (((0, 0, 0), (1, 0, 1)), ((0, 0, -1), (0, 0, 0), (0, 0, 0)), ((1, 0, 1), (-1, 0, -1))),
    (((0, 1, 1), (0, 1, 1)), ((0, 0, 0), (0, 0, 0), (0, 1, 0)), ((0, 0, 0), (0, 1, 1))),
)
_HK_MIX = sorted({tuple(o[g][c] for _, _, o in _HK_AHEAD) for g in range(2) for c in range(3)}, reverse=True)
_HK_MIX_OF = [[_HK_MIX.index(tuple(o[g][c] for _, _, o in _HK_AHEAD)) for c in range(3)] for g in range(2)]


def _flat(rows):
    return [c for row in rows for c in row]


def _signed_sum(coefs, values):
    terms = sorted(((c, i) for i, c in enumerate(coefs) if c), key=lambda t: -t[0])
    acc = values[terms[0][1]] if terms[0][0] > 0 else -values[terms[0][1]]
    for c, i in terms[1:]:
        acc = acc + values[i] if c > 0 else acc - values[i]
    return acc


def _strassen_lhs(a11, a12, a21, a22):
    return [a11 + a22, a21 + a22, a11, a22, a11 + a12, a21 - a11, a12 - a22]


def _strassen_rhs(b11, b12, b21, b22):
    return [b11 + b22, b11, b12 - b22, b21 - b11, b22, b11 + b12, b21 + b22]


def _strassen_out(m1, m2, m3, m4, m5, m6, m7):
    return m1 + m4 - m5 + m7, m3 + m5, m2 + m4, m1 - m2 + m3 + m6


def _split_pair(words):
    return pltpu.bitcast(words << 16, F32), pltpu.bitcast(words & jnp.uint32(0xFFFF0000), F32)


def _stack_bf16(a, b):
    return jnp.concatenate([a, b], axis=0).astype(BF16)


def _tiles(ref, lead, indices, axis):
    words = ref.bitcast(U32)
    return pltpu.bitcast(jnp.concatenate([words[(*lead, i)] for i in indices], axis=axis), BF16)


def _low_lanes(rows):
    return lax.broadcasted_iota(jnp.int32, (rows, TILE), 1) < TILE // 2


def _make_kernel(S, D, H, E, M, SEG, F):
    NP = H // 2
    NC = D // TILE
    DM = NC * TILE
    L = M + SEG
    G = L // 8
    SPB = TILE // SEG
    NB = S // TILE
    NS = S // SEG
    UNITS = 2 * H + NP
    ZL = 2 * CHUNK
    XL = ZL // SPB + 1
    S1 = NS - CHUNK
    KL = CHUNK // SPB * TILE
    RC = D // SPB
    DH, FH, SH = D // 2, F // 2, S // 2
    FLUSH = (3, 5, 7, 8)
    scale = E ** -0.5 * math.log2(math.e)

    def kernel(xT_h, mem_h, wq_h, wk_h, wv_h, woT_h, w1_h, b1_h, w2_h, b2_h, out_h,
               X, WA, b2_s, WS, mem_s, B2, hT, b1_s, NS_, out_s, KT, GA, unscale, GX, w2_s, w1_s, O, VT, AH,
               narrow, WC, wk_s, wo_s, wq_s, U, HS, nT, KX, xT_s, Z, wv_s,
               sem_q, sem_k, sem_v, sem_o, sem_m, sem_out):
        wq_u, wk_u, wv_u = (r.bitcast(U32) for r in (wq_h, wk_h, wv_h))

        def k_copies(p):
            return [pltpu.make_async_copy(wq_u.at[:, p, :], wq_s.at[p], sem_q.at[p]),
                    pltpu.make_async_copy(wk_u.at[:, p, :], wk_s.at[p], sem_k.at[p])]

        def v_copies(p):
            return [pltpu.make_async_copy(wv_u.at[:, p, :], wv_s.at[p], sem_v.at[p]),
                    pltpu.make_async_copy(woT_h.at[pl.ds(2 * p, 2)], wo_s.at[pl.ds(2 * p, 2)], sem_o.at[p])]

        def x_copy(b0, b1, sem):
            cols = pl.ds(b0 * TILE, (b1 - b0) * TILE)
            return pltpu.make_async_copy(xT_h.at[:, cols], xT_s.at[:, cols], sem)

        cp_x0 = x_copy(0, 3, sem_m.at[0])
        cp_x1 = x_copy(3, XL, sem_m.at[1])
        cp_x2 = x_copy(XL, NB, sem_m.at[2])
        cp_mem = pltpu.make_async_copy(mem_h, mem_s, sem_m.at[3])
        cp_b1 = pltpu.make_async_copy(b1_h, b1_s, sem_m.at[4])
        cp_b2 = pltpu.make_async_copy(b2_h, b2_s, sem_m.at[5])
        cp_w1 = pltpu.make_async_copy(w1_h, w1_s, sem_m.at[6])
        cp_w2 = pltpu.make_async_copy(w2_h, w2_s, sem_m.at[7])
        small = [cp_x0, cp_mem, cp_b1, cp_b2]
        for cp in small:
            cp.start()
        for p in range(NP):
            for cp in k_copies(p):
                cp.start()
        cp_x1.start()
        for p in range(NP):
            for cp in v_copies(p):
                cp.start()
        cp_x2.start()

        lane = lax.broadcasted_iota(jnp.int32, (8, TILE), 1)
        row = lax.broadcasted_iota(jnp.int32, (8, TILE), 0)
        low = lane < TILE // 2

        def transpose_x(src, dst, j):
            r0 = pl.multiple_of(j * TILE, 64)
            r1 = pl.multiple_of(jnp.minimum(j * TILE + 64, DM), 64)
            t = jnp.concatenate([xT_s[pl.ds(r0, 64), pl.ds(src, TILE)], xT_s[pl.ds(r1, 64), pl.ds(src, TILE)]], axis=0)
            X[j, pl.ds(dst, TILE), :] = t.astype(F32).T

        def layernorm(tiles):
            mask = _low_lanes(tiles[0].shape[0])

            def mean(ts):
                acc = functools.reduce(jnp.add, ts[:NC]) + jnp.where(mask, ts[NC], 0.0)
                return jnp.sum(acc, axis=1, keepdims=True) * (1.0 / D)

            m = mean(tiles)
            c = [t - m for t in tiles]
            r = lax.rsqrt(mean([t * t for t in c]) + EPS)
            return [t * r for t in c]

        def normalize_x(src, dst, rows):
            z = layernorm([X[c, pl.ds(src, rows), :] for c in range(NC + 1)])
            for c in range(NC + 1):
                Z[c, pl.ds(dst, rows), :] = z[c]

        def residual(t0, slot, dst_slot, dst):
            h = [X[c, pl.ds(t0, SEG), :] + O[slot, c] for c in range(NC + 1)]
            for c in range(NC + 1):
                HS[dst_slot, c, pl.ds(dst, SEG), :] = h[c]
            n = layernorm(layernorm(h))
            for c in range(NC + 1):
                NS_[dst_slot, c, pl.ds(dst, SEG), :] = n[c]

        def transpose_back(dst, src, slot, col, j):
            dst[pl.ds(pl.multiple_of(j * TILE, TILE), TILE), pl.ds(col, TILE)] = src[slot, j].T

        def ahead_weights(units):
            return [_tiles(WA, (r,), units, 1) for r in range(len(_HK_AHEAD))]

        def ahead(chunk, units, weights, after=lambda v: v):
            base = pl.multiple_of(chunk * CHUNK * SEG, CHUNK * SEG)
            x = [jnp.concatenate([Z[k, pl.ds(base + n * SEG + SEG - 16 + 8 * g, 8), :] for n in range(CHUNK)], axis=0)
                 for g in range(2) for k in range(NC)]
            m = [_dot(after(_signed_sum(_flat(coefs), x)), w) for w, (coefs, _, _) in zip(weights, _HK_AHEAD)]
            for n, coefs in enumerate(_HK_MIX):
                v = _signed_sum(coefs, m)
                for i, unit in enumerate(units):
                    AH[chunk & 1, unit, n] = v[:, TILE * i:TILE * (i + 1)]

        def store_unit(cols, unit):
            blocks = [col[TILE * k:TILE * (k + 1)] for k in range(NC) for col in cols]
            for W, table in ((WS, _HK_STEP), (WA, _HK_AHEAD)):
                for r, (_, coefs, _) in enumerate(table):
                    W[r, unit] = _signed_sum(_flat(coefs), blocks).astype(BF16)

        def store_head(y, unit):
            store_unit([y[:, TILE * c:TILE * (c + 1)] for c in range(NC)], unit)

        def fold(l0, l1, r0, r1, late=lambda a: a):
            def operands(l, r):
                a = jnp.concatenate([l[DM:], l[:DM]], axis=0)
                left = _strassen_lhs(a[:DH, :TILE], a[:DH, TILE:], a[DH:, :TILE], a[DH:, TILE:])
                right = _strassen_rhs(r[:TILE, :TILE], r[TILE:2 * TILE, :TILE], r[:TILE, TILE:], r[TILE:2 * TILE, TILE:])
                return a.astype(BF16), [v.astype(BF16) for v in left], [v.astype(BF16) for v in right]

            def two_tiles(left, right):
                c = _strassen_out(*[_dot_nt(x, y) for x, y in zip(left, right)])
                return jnp.concatenate([jnp.concatenate(c[:2], axis=1), jnp.concatenate(c[2:], axis=1)], axis=0)

            def rest(n0, n1):
                return jnp.concatenate([_dot_nt(r[DM:].astype(BF16), l[n0:n1].astype(BF16))
                                        for l, r in ((l0, r0), (l1, r1))], axis=0)

            a0, left0, right0 = operands(l0, r0)
            a1, left1, right1 = operands(l1, r1)
            y0a = two_tiles(left0, right0)
            y0b = _dot_nt(a0, r0[2 * TILE:DM].astype(BF16))
            y1b = _dot_nt(late(a1), r1[2 * TILE:DM].astype(BF16))
            ta = rest(0, 2 * TILE)
            tb = rest(2 * TILE, D)
            y1a = two_tiles(left1, right1)
            t = jnp.concatenate([ta, tb, jnp.zeros((TILE, 64), F32)], axis=1)
            return jnp.concatenate([y0a, y0b], axis=1), jnp.concatenate([y1a, y1b], axis=1), t

        def magnitude(x):
            m = functools.reduce(jnp.maximum, [jnp.abs(x[r:r + 8]) for r in range(0, x.shape[0], 8)])
            m = jnp.max(jnp.max(m, axis=0, keepdims=True), axis=1, keepdims=True)
            m = pltpu.bitcast(jnp.broadcast_to(m, (8, TILE)), U32) & jnp.uint32(0x7F800000)
            return jnp.clip(pltpu.bitcast(m, F32), 2.0 ** -60, 2.0 ** 60)

        def store_narrow(p):
            tk, tq, tv = narrow[p, 0], narrow[p, 1], narrow[p, 2]
            mk, mv = magnitude(tk), magnitude(tv)
            unscale[p] = mv / mk
            store_unit([tk, tv * (mk / mv)[:1], tq], 2 * H + p)

        def fold_keys(p, _):
            for cp in k_copies(p):
                cp.wait()
            before = jnp.maximum(p - 1, 0)
            units = (2 * before, 2 * before + 1)
            weights = ahead_weights(units)
            y0, y1, t = fold(*_split_pair(wk_s[p]), *_split_pair(wq_s[p]))
            narrow[p, 0] = t[:, :DM].T
            WC[p] = (t[:64, DM:] + pltpu.roll(t[64:, DM:], 64, 1)).astype(BF16)
            store_head(y0[64:], 2 * p)
            store_head(y1[64:], 2 * p + 1)
            narrow[p, 1] = jnp.concatenate([y0[:64], y1[:64]], axis=0).T
            b1 = b1_s[...].astype(F32)
            rows = lax.broadcasted_iota(jnp.int32, b1.shape, 0)
            per = pl.cdiv(F // TILE, NP)
            for k in range(per):
                r = jnp.minimum(p * per + k, F // TILE - 1)
                bias = jnp.sum(jnp.where(rows == r, b1, 0.0), axis=0, keepdims=True)
                U[:, pl.ds(pl.multiple_of(r * TILE, TILE), TILE)] = jnp.broadcast_to(bias, (D, TILE))
            ahead(0, units, weights)

        def fold_values(p, _):
            for cp in v_copies(p):
                cp.wait()
            store_narrow(jnp.maximum(p - 1, 0))
            probe = WA[0, p, 0:16, :]
            units = (H + 2 * p - 2, H + 2 * p - 1)
            weights = ahead_weights(units)

            def late(a):
                keep = lax.broadcasted_iota(jnp.int32, (16, TILE), 1) < p + TILE
                head = jnp.concatenate([jnp.where(keep, a[:16, :TILE], probe), a[:16, TILE:]], axis=1)
                return jnp.concatenate([head, a[16:]], axis=0)

            y0, y1, t = fold(*_split_pair(wv_s[p]), wo_s[2 * p].astype(F32),
                             wo_s[2 * p + 1].astype(F32), late)
            t = t.T
            narrow[p, 2] = t[:DM]
            store_head(y0[64:], H + 2 * p)
            store_head(y1[64:], H + 2 * p + 1)
            m = _low_lanes(64)
            top = jnp.concatenate([y0[:64], jnp.where(m, t[DM:D], 0.0)], axis=1)
            bot = jnp.concatenate([y1[:64], jnp.where(m, 0.0, t[DM:D])], axis=1)
            b2 = _stack_bf16(top, bot)
            for c in range(NC + 1):
                B2[c, p] = b2[:, TILE * c:TILE * (c + 1)]
            ahead(0, units, weights)
            r = pl.multiple_of((CHUNK + p) * SEG, SEG)
            normalize_x(r, r, SEG)
            c0 = pl.multiple_of((3 + (p >> 2)) * TILE, TILE)
            transpose_x(c0, c0, p & 3)

        O[...] = jnp.zeros(O.shape, F32)
        HS[1] = jnp.zeros(HS.shape[1:], F32)
        NS_[...] = jnp.zeros(NS_.shape, F32)
        hT[0:TILE, 0:TILE] = jnp.zeros((TILE, TILE), F32)
        nT[0:TILE, 0:TILE] = jnp.zeros((TILE, TILE), F32)
        narrow[0, 2] = jnp.zeros((DM, TILE), F32)
        WA[:, 0:2] = jnp.zeros((len(_HK_AHEAD), 2, TILE, TILE), BF16)

        for cp in small:
            cp.wait()
        for b in range(3):
            for j in range(NC + 1):
                transpose_x(b * TILE, b * TILE, j)
            if b < 2:
                normalize_x(b * TILE, b * TILE, TILE)
        lax.fori_loop(0, NP, fold_keys, None)
        cp_x1.wait()
        lax.fori_loop(0, NP, fold_values, None)
        store_narrow(NP - 1)
        for units in ((2 * H - 2, 2 * H - 1), range(2 * H, 2 * H + NP // 2), range(2 * H + NP // 2, UNITS)):
            ahead(0, units, ahead_weights(units))

        causal = row >= (lane & 7)
        pair_of_lane = lane >> 4

        def over_keys(x, op):
            for k in (1, 2, 4):
                x = op(x, jnp.where((lane & k) != 0, pltpu.roll(x, k, 1), pltpu.roll(x, TILE - k, 1)))
            return x

        def queries_of(t):
            return [0] + list(range(max(t, 1), G))

        def keys_of(r):
            return G if r == 0 else r + 1

        def segment(i, s, mem, fill_mid, fill_end, run_ahead):
            t0 = pl.multiple_of(s * SEG, SEG)
            zt = [jnp.concatenate([mem[:, TILE * c:TILE * (c + 1)], Z[c, pl.ds(t0, SEG), :]], axis=0)
                  for c in range(NC + 1)]
            zs = jnp.concatenate(zt, axis=1)
            shared = [v[L - 16:L - 8] for v in zt[:NC]] + [v[L - 8:] for v in zt[:NC]]
            lhs = [jnp.concatenate([_signed_sum(coefs[0], [v[:L - 16] for v in zt[:NC]]),
                                    _signed_sum(_flat(coefs), shared)], axis=0).astype(BF16)
                   for coefs, _, _ in _HK_STEP]
            early = lambda unit, n: AH[(s >> 3) & 1, unit, n, pl.ds(pl.multiple_of((s & 7) * 8, 8), 8), :]
            g = [_stack_bf16(jnp.where(low, zt[NC][8 * t:8 * t + 8], 0.0), jnp.where(low, 0.0, zt[NC][8 * t:8 * t + 8]))
                 for t in range(G)]
            zero = jnp.zeros((16, TILE), BF16)
            tails = [jnp.concatenate([g[(b - p) % NP] if (b - p) % NP < G else zero for b in range(NP)], axis=0)
                     for p in range(NP)]

            keep = lane < i + TILE
            pinned = []
            slot = (i >> 1) & 1
            some_rows = pl.ds(pl.multiple_of(((i >> 2) & (TILE // 8 - 1)) * 8, 8), 8)

            def after(a):
                if not pinned:
                    return a
                wide = a.astype(F32)
                head = wide[:8, :TILE]
                for v in pinned:
                    head = jnp.where(keep, head, v)
                pinned.clear()
                if a.shape[1] > TILE:
                    head = jnp.concatenate([head, wide[:8, TILE:]], axis=1)
                return jnp.concatenate([head, wide[8:]], axis=0).astype(a.dtype)

            def project(unit):
                m = [_dot(after(a), _tiles(WS, (r,), (unit, unit + 1), 1)) for r, a in enumerate(lhs)]
                last = [v[L - 16:] for v in m]
                out = []
                for c in range(NC):
                    y = _signed_sum([o[0][c] for _, _, o in _HK_STEP], m)
                    u = _signed_sum([o[1][c] for _, _, o in _HK_STEP], last)
                    out.append([[y[8 * t:8 * t + 8, TILE * k:TILE * (k + 1)] for t in range(G - 2)]
                                + [y[L - 16:, TILE * k:TILE * (k + 1)] + early(unit + k, _HK_MIX_OF[0][c]),
                                   u[:, TILE * k:TILE * (k + 1)] + early(unit + k, _HK_MIX_OF[1][c])]
                                for k in range(2)])
                return out

            def project_heads(T, first, p0, p1):
                for p in range(p0, p1):
                    for c, (even, odd) in enumerate(project(first + 2 * p)):
                        for t in range(G):
                            T[c, t * TILE + 16 * p:t * TILE + 16 * (p + 1), :] = _stack_bf16(even[t], odd[t])

            q_tail = [None] * NP

            def project_narrow(j0, j1):
                for j in range(j0, j1):
                    k3, v3, q = project(2 * H + 2 * j)
                    for k in range(2):
                        p = 2 * j + k
                        q_tail[p] = jnp.concatenate(q[k], axis=0)
                        for T, rows in ((KT, k3[k]), (VT, [v * unscale[p] for v in v3[k]])):
                            for t, v in enumerate(rows):
                                T[NC, t * TILE + 16 * p:t * TILE + 16 * (p + 1), :] = _stack_bf16(
                                    jnp.where(low, v, 0.0), jnp.where(low, 0.0, v))

            def transpose_keys(c):
                KX[c] = pltpu.bitcast(pltpu.bitcast(KT.bitcast(U32)[c], BF16).T, U32)

            b, j = s >> 2, s & 3
            col = lambda blk: pl.multiple_of(jnp.clip(blk, 0, NB - 1) * TILE, TILE)
            sp = s - 1

            project_heads(KT, 0, 0, 2)
            g0 = pltpu.bitcast(tails[0].T, U32)
            for p in range(NP):
                GX[p] = pltpu.roll(g0, 16 * p, 1) if p else g0
            residual(pl.multiple_of(jnp.maximum(sp, 0) * SEG, SEG), sp & 3, (sp >> 2) & 1,
                     pl.multiple_of((sp & 3) * SEG, SEG))
            project_heads(KT, 0, 2, 5)
            pinned.append(NS_[slot, 0, some_rows, :])
            project_heads(KT, 0, 5, NP)
            for c in range(NC):
                transpose_keys(c)
            project_narrow(0, 3)
            pinned.append(pltpu.bitcast(KX[0, 56:64, TILE * (G - 1):], F32))
            project_narrow(3, NP // 2)
            transpose_keys(NC)
            q2 = jnp.concatenate(q_tail, axis=1) + _dot(after(zt[NC])[:, :64], _tiles(WC, (), range(NP), 1))
            pinned.append(pltpu.bitcast(KX[1, 56:64, TILE * (G - 1):], F32))
            fill_mid(after, lambda: pinned.append(pltpu.bitcast(GX[NP - 1, 56:64, :], F32)))

            o = [_dot(after(q2[:, TILE * p:TILE * (p + 1)]), pltpu.bitcast(GX[p], BF16)) for p in range(NP)]
            extra = []
            for r in range(G):
                extra.append([])
                for t in range(keys_of(r)):
                    x = o[0][8 * r:8 * r + 8]
                    for p in range(1, NP):
                        x = jnp.where(pair_of_lane == (p + t) % NP, o[p][8 * r:8 * r + 8], x)
                    extra[r].append(pltpu.roll(x, TILE - 16 * t, 1) if t else x)
            scores = {}
            for t in range(G):
                rs = queries_of(t)
                a = after(jnp.concatenate([zs[8 * r:8 * r + 8] for r in rs], axis=0))
                y = _dot(a, jnp.concatenate([pltpu.bitcast(KX[c, :, TILE * t:TILE * (t + 1)], BF16)
                                             for c in range(NC + 1)], axis=0))
                for n, r in enumerate(rs):
                    scores[r, t] = y[8 * n:8 * n + 8]
            probs = []
            for r in range(G):
                tiles = [scores[r, t] + extra[r][t] for t in range(keys_of(r))]
                if r > 0:
                    tiles[r] = jnp.where(causal, tiles[r], -1e9 * math.sqrt(E))
                m = over_keys(functools.reduce(jnp.maximum, tiles), jnp.maximum)
                e = [jnp.exp2((x - m) * scale) for x in tiles]
                total = over_keys(functools.reduce(jnp.add, e), jnp.add)
                inv = pl.reciprocal(total, approx=True)
                inv = inv * (2.0 - total * inv)
                probs.append([x * inv for x in e])

            project_heads(VT, H, 0, NP - 1)
            rotated = [[pltpu.roll(x, 16 * t, 1) if t else x for t, x in enumerate(tiles)] for tiles in probs]
            pz = []
            for p in range(NP):
                rows = []
                for r in range(G):
                    n = keys_of(r)
                    x = rotated[r][0] if n == G else jnp.where(pair_of_lane == p, rotated[r][0], 0.0)
                    for t in range(1, n):
                        x = jnp.where(pair_of_lane == (p + t) % NP, rotated[r][t], x)
                    rows.append(x)
                pz.append(_dot(after(jnp.concatenate(rows, axis=0)), tails[p]))
            project_heads(VT, H, NP - 1, NP)
            transpose_back(nT, NS_, 1 - (b & 1), col(b - 1), j)
            if run_ahead:
                normalize_x(pl.multiple_of(jnp.minimum(s + ZL, NS - 1) * SEG, SEG),
                            pl.multiple_of(jnp.minimum(s + ZL, NS) * SEG, SEG), SEG)
            transpose_back(hT, HS, 1 - (b & 1), col(b - 1), j)
            if run_ahead:
                transpose_x(col(b + XL), pl.multiple_of(jnp.minimum(b + XL, NB) * TILE, TILE), j)
            y = _dot(after(jnp.concatenate(pz, axis=1)),
                     jnp.concatenate([_tiles(B2, (c,), range(NP), 0) for c in range(NC + 1)], axis=1))
            out = [y[8 * r:8 * r + 8] for r in range(G)]
            if run_ahead:
                pinned.extend([Z[i & 3, some_rows, :], nT[some_rows, 0:TILE]])
            else:
                pinned.extend([nT[some_rows, 0:TILE], hT[some_rows, 0:TILE]])
            for t in range(G):
                rs = queries_of(t)
                a = after(jnp.concatenate([probs[r][t] for r in rs], axis=0))
                y = _dot(a, jnp.concatenate([pltpu.bitcast(VT.bitcast(U32)[c, 64 * t:64 * t + 64, :], BF16)
                                             for c in range(NC + 1)], axis=1))
                for n, r in enumerate(rs):
                    out[r] = out[r] + y[8 * n:8 * n + 8]
            if run_ahead:
                pinned.extend([hT[some_rows, 0:TILE], X[i & 3, some_rows, :]])
            fill_end(after)

            out = jnp.concatenate(out, axis=0)
            tail = out[:, DM:]
            out = jnp.concatenate([out[:, :DM], tail + pltpu.roll(tail, 64, 1)], axis=1)
            for c in range(NC + 1):
                O[s & 3, c] = out[M:, TILE * c:TILE * (c + 1)]
            return out[:M]

        def two_segments(i, mem):
            first = (i & 3) * (UNITS // 4)
            for n in range(2):
                s = 2 * i + n

                def work(at, after):
                    units = (first + at, first + at + 1)
                    ahead((s >> 3) + 1, units, ahead_weights(units), after)

                def fill_mid(after, pin):
                    work(4 * n + 2, after)
                    pin()
                    if n == 0:
                        work(8, after)

                mem = segment(i, s, mem, fill_mid, functools.partial(work, 4 * n), True)
            return mem

        def two_last_segments(i, mem):
            for n in range(2):
                k0 = pl.multiple_of(((2 * i + n) >> 2) * TILE, TILE)
                r0 = pl.multiple_of(((2 * i + n) & 3) * RC, 8)

                def mix(c0, c1, after):
                    U[pl.ds(r0, RC), c0:c1] += _dot(after(nT[pl.ds(r0, RC), pl.ds(k0, TILE)]), w1_s[pl.ds(k0, TILE), c0:c1])

                def fill_mid(after, pin):
                    mix(0, 6 * TILE, after)
                    pin()

                mem = segment(i, S1 + 2 * i + n, mem, fill_mid, functools.partial(mix, 6 * TILE, F), False)
            return mem

        cp_x2.wait()
        cp_w1.start()
        cp_w2.start()
        mem = mem_s[...].astype(F32)
        mem = jnp.concatenate([mem, mem[:, DM:]], axis=1)
        mem = lax.fori_loop(0, S1 // 2, two_segments, mem)
        cp_w1.wait()
        lax.fori_loop(0, CHUNK // 2, two_last_segments, mem)
        cp_w2.wait()

        def strassen_operands(w, r0, rh, c0, ch):
            return _strassen_rhs(*[w[r0 + dr:r0 + dr + rh, c0 + dc:c0 + dc + TILE].astype(F32)
                                   for dr in (0, rh) for dc in (0, ch)])

        last = (NB - 1) & 1
        KH = (S - KL) // 2
        residual((NS - 1) * SEG, (NS - 1) & 3, last, (SPB - 1) * SEG)
        a11, a21 = nT[:DH, KL:KL + KH], nT[DH:D, KL:KL + KH]
        a3, a6 = a11.astype(BF16), (a21 - a11).astype(BF16)
        for t in range(0, FH, TILE):
            w = strassen_operands(w1_s, KL, KH, t, FH)
            m3 = _dot(a3, w[2].astype(BF16))
            U[:DH, FH + t:FH + t + TILE] += m3
            U[DH:, FH + t:FH + t + TILE] += m3 + _dot(a6, w[5].astype(BF16))
        for dst, src in ((nT, NS_), (hT, HS)):
            for j in range(NC + 1):
                transpose_back(dst, src, last, (NB - 1) * TILE, j)
        a = [v.astype(BF16) for v in _strassen_lhs(a11, nT[:DH, KL + KH:], a21, nT[DH:D, KL + KH:])]
        for t in range(0, FH, TILE):
            w = strassen_operands(w1_s, KL, KH, t, FH)
            m1, m2, m4, m5, m7 = (_dot(a[k], w[k].astype(BF16)) for k in (0, 1, 3, 4, 6))
            u = (U[:DH, t:t + TILE] + (m1 + m4 - m5 + m7), U[:DH, FH + t:FH + t + TILE] + m5,
                 U[DH:, t:t + TILE] + (m2 + m4), U[DH:, FH + t:FH + t + TILE] + (m1 - m2))
            for k, v in enumerate(_strassen_lhs(*[jax.nn.gelu(v, approximate=True) for v in u])):
                GA[k, :, t:t + TILE] = v

        b2 = b2_s[...].astype(F32)
        copies = []
        for f, (n0, n1) in enumerate(zip((0,) + FLUSH[:-1], FLUSH)):
            for n in range(n0, n1):
                w = strassen_operands(w2_s, 0, FH, n * TILE, SH)
                m = [_dot(GA[k].astype(BF16), w[k].astype(BF16)) for k in range(7)]
                for q, y in enumerate(_strassen_out(*m)):
                    rs = slice((q >> 1) * DH, (q >> 1) * DH + DH)
                    tile = (q & 1) * (SH // TILE) + n
                    cs = slice(tile * TILE, (tile + 1) * TILE)
                    out_s[rs, cs] = (y + b2[tile:tile + 1] + hT[rs, cs]).astype(BF16)
            for half in range(2):
                cols = pl.ds(half * SH + n0 * TILE, (n1 - n0) * TILE)
                copies.append(pltpu.make_async_copy(out_s.at[:, cols], out_h.at[:, cols], sem_out.at[2 * f + half]))
                copies[-1].start()
        for cp in copies:
            cp.wait()

    return kernel


@functools.partial(jax.jit, static_argnames=("A_seg_len",))
def pallas_sequential_preLN__memory_aug_recurrent_mem_tr__mixer_token_mlp__prompt_kernel(
    A_x, A_mem0, A_Wq, A_Wk, A_Wv, A_Wo, A_seg_len, B_x, B_w1, B_b1, B_w2, B_b2,
):
    del B_x
    B, S, D = A_x.shape
    M = A_mem0.shape[1]
    H, E = A_Wq.shape[1:]
    F = B_w1.shape[1]
    SEG = int(A_seg_len)
    assert (B, S, D, M, H, E, F, SEG) == (1, 2048, 448, 8, 16, 256, 1792, 32), "the tiling is laid out for these sizes"
    NP = H // 2
    NC = D // TILE
    DM = NC * TILE
    LT = (M + SEG) // 8 * TILE
    UNITS = 2 * H + NP
    vmem = pltpu.VMEM
    dma = pltpu.SemaphoreType.DMA
    in_hbm = pl.BlockSpec(memory_space=pl.ANY)
    outT = pl.pallas_call(
        _make_kernel(S, D, H, E, M, SEG, F),
        in_specs=[in_hbm] * 10,
        out_specs=in_hbm,
        out_shape=jax.ShapeDtypeStruct((D, S), A_x.dtype),
        scratch_shapes=[
            vmem((NC + 1, S + TILE, TILE), F32),
            vmem((len(_HK_AHEAD), UNITS, TILE, TILE), BF16),
            vmem((S // TILE, TILE), BF16),
            vmem((len(_HK_STEP), UNITS, TILE, TILE), BF16),
            vmem((M, D), BF16),
            vmem((NC + 1, NP, TILE, TILE), BF16),
            vmem((DM + TILE, S), F32),
            vmem((F // TILE, TILE), BF16),
            vmem((2, NC + 1, TILE, TILE), F32),
            vmem((D, S), BF16),
            vmem((NC + 1, LT, TILE), BF16),
            vmem((7, D // 2, F // 2), F32),
            vmem((NP, 8, TILE), F32),
            vmem((NP, 64, TILE), U32),
            vmem((F, S), BF16),
            vmem((S, F), BF16),
            vmem((4, NC + 1, SEG, TILE), F32),
            vmem((NC + 1, LT, TILE), BF16),
            vmem((2, UNITS, len(_HK_MIX), CHUNK * 8, TILE), F32),
            vmem((NP, 3, DM, TILE), F32),
            vmem((NP, 64, TILE), BF16),
            vmem((NP, D, E), U32),
            vmem((H, D, E), BF16),
            vmem((NP, D, E), U32),
            vmem((D, F), F32),
            vmem((2, NC + 1, TILE, TILE), F32),
            vmem((DM + TILE, S), F32),
            vmem((NC + 1, 64, LT), U32),
            vmem((D, S), BF16),
            vmem((NC + 1, S + SEG, TILE), F32),
            vmem((NP, D, E), U32),
            dma((NP,)), dma((NP,)), dma((NP,)), dma((NP,)), dma((8,)), dma((8,)),
        ],
        compiler_params=pltpu.CompilerParams(vmem_limit_bytes=110 * 1024 * 1024),
    )(jnp.swapaxes(A_x.reshape(S, D), 0, 1), A_mem0.reshape(M, D), A_Wq, A_Wk, A_Wv, jnp.swapaxes(A_Wo, 1, 2),
      B_w1, B_b1.reshape(F // TILE, TILE), B_w2, B_b2.reshape(S // TILE, TILE))
    return jnp.swapaxes(outT, 0, 1).reshape(B, S, D)
```
